```python
import os as _os
_os.environ.setdefault("JAX_PLATFORMS", "cpu")
import jax
import jax.numpy as jnp

def _softmax(x, axis=-1):
    return jax.nn.softmax(x, axis=axis)
def _gelu(x):
    return jax.nn.gelu(x, approximate=True)
def _silu(x):
    return jax.nn.silu(x)
def _sigmoid(x):
    return jax.nn.sigmoid(x)
def _layernorm(x, axis=-1, eps=1e-5):
    m = jnp.mean(x, axis=axis, keepdims=True)
    v = jnp.var(x, axis=axis, keepdims=True)
    return (x - m) / jnp.sqrt(v + eps)
def _scatter_add(tgt, idx, src, axis=0):
    return tgt.at[idx].add(src)
def _segment_sum(src, seg, n):
    return jax.ops.segment_sum(src, seg, n)
class _Rng:
    def __init__(self, key):
        self._k = key
    def _next(self):
        self._k, sub = jax.random.split(self._k)
        return sub
    def normal(self, shape):
        return jax.random.normal(self._next(), shape, dtype=jnp.bfloat16)
    def randint(self, lo, hi, shape):
        return jax.random.randint(self._next(), shape, lo, hi, dtype=jnp.int32)
    def uniform(self, shape, lo=0.0, hi=1.0):
        return jax.random.uniform(self._next(), shape, jnp.bfloat16, lo, hi)
    def permutation(self, n):
        return jax.random.permutation(self._next(), n)


kernel_name = 'interleave_layers__linear_kernel_hedgehog__ssm_conv_s4__prompt'

def setup_inputs():
    _rng = _Rng(jax.random.key(int.from_bytes(__import__("os").urandom(4), "little")))
    _w = (lambda a: (lambda t: t.astype(jnp.bfloat16) if jnp.issubdtype(t.dtype, jnp.floating) else t)(jnp.asarray(a)))
    def _A_setup():
        B, S, D, H = 1, 2048, 512, 32
        Dh = D // H
        return {
            "x": _w((lambda *s: _rng.normal(s) * 0.05)(B, S, D)),
            "wqkv": _w((lambda *s: _rng.normal(s) * 0.4)(D, 3 * D)),
            "w_phi": _w((lambda *s: _rng.normal(s) * 0.4)(H, Dh, Dh) * (Dh ** -0.5)),
            "wo": _w((lambda *s: _rng.normal(s) * 0.05)(D, D)),
        }
    _A_in = _A_setup()

    def _B_setup():
        B, L, D, N = 1, 2048, 512, 128
        A_re = -jnp.exp((lambda *s: _rng.normal(s) * 0.2)(D, N))
        A_im = jnp.pi * (lambda *s: _rng.normal(s) * 0.2)(D, N)
        B_re = (lambda *s: _rng.normal(s) * 0.2)(D, N)
        B_im = (lambda *s: _rng.normal(s) * 0.2)(D, N)
        C_re = (lambda *s: _rng.normal(s) * 0.2)(D, N)
        C_im = (lambda *s: _rng.normal(s) * 0.2)(D, N)
        log_dt = (lambda *s: _rng.normal(s) * 0.2)(D) * 0.5 - 4.0
        Dskip = (lambda *s: _rng.normal(s) * 0.2)(D)
        return {
            "u": _w((lambda *s: _rng.normal(s) * 0.05)(B, L, D)),
            "A_re": _w(A_re),
            "A_im": _w(A_im),
            "B_re": _w(B_re),
            "B_im": _w(B_im),
            "C_re": _w(C_re),
            "C_im": _w(C_im),
            "log_dt": _w(log_dt),
            "Dskip": _w(Dskip),
        }
    _B_in = _B_setup()

    return {
        "A_x": _A_in["x"],
        "A_wqkv": _A_in["wqkv"],
        "A_w_phi": _A_in["w_phi"],
        "A_wo": _A_in["wo"],
        "B_u": _B_in["u"],
        "B_A_re": _B_in["A_re"],
        "B_A_im": _B_in["A_im"],
        "B_B_re": _B_in["B_re"],
        "B_B_im": _B_in["B_im"],
        "B_C_re": _B_in["C_re"],
        "B_C_im": _B_in["C_im"],
        "B_log_dt": _B_in["log_dt"],
        "B_Dskip": _B_in["Dskip"],
    }

def reference(A_x, A_wqkv, A_w_phi, A_wo, B_u, B_A_re, B_A_im, B_B_re, B_B_im, B_C_re, B_C_im, B_log_dt, B_Dskip):
    def _A_ref(x, wqkv, w_phi, wo):
        B, S, D = x.shape
        H = 32; Dh = D // H
        qkv = (lambda x, *d: x.transpose(*d))((x @ wqkv).reshape(B, S, 3, H, Dh), 2, 0, 3, 1, 4)
        q, k, v = qkv[0], qkv[1], qkv[2]
        pq = jnp.einsum("bhsd,hdf->bhsf", q, w_phi)
        pk = jnp.einsum("bhsd,hdf->bhsf", k, w_phi)
        phi_q = jnp.concatenate([_softmax(pq, axis=-1), _softmax(-pq, axis=-1)], axis=-1)
        phi_k = jnp.concatenate([_softmax(pk, axis=-1), _softmax(-pk, axis=-1)], axis=-1)
        kv = jnp.einsum("bhsf,bhsd->bhfd", phi_k, v)
        z  = jnp.einsum("bhsf->bhf", phi_k)
        num = jnp.einsum("bhqf,bhfd->bhqd", phi_q, kv)
        den = jnp.einsum("bhqf,bhf->bhq", phi_q, z)[..., None] + 1e-6
        o = num / den
        return (lambda x, *d: x.transpose(*d))(o, 0, 2, 1, 3).reshape(B, S, D) @ wo

    def _B_ref(u, A_re, A_im, B_re, B_im, C_re, C_im, log_dt, Dskip):
        Bsz, L, D = u.shape
        dt = jnp.exp(log_dt)[:, None]
        A = A_re + 1j * A_im
        Bc = B_re + 1j * B_im
        Cc = C_re + 1j * C_im
        logdA = dt * A
        dB = dt * Bc
        l = (lambda x, dt: x.astype(dt))(jnp.arange(L), A_re.dtype)
        P = jnp.exp(logdA[:, :, None] * l[None, None, :])
        K = jnp.einsum("dn,dnl,dn->dl", Cc, P, dB).real
        L2 = 2 * L
        Kp = jnp.pad(K, ((0, 0), (0, L)))
        up = (lambda x, *d: x.transpose(*d))(u, 0, 2, 1)
        up = jnp.pad(up, ((0, 0), (0, 0), (0, L)))
        Kf = (lambda x, axes=(-2,-1): jnp.fft.rfft2(x.astype(jnp.float32), axes=axes))(Kp[:, None, :], axes=(-2, -1))
        Uf = (lambda x, axes=(-2,-1): jnp.fft.rfft2(x.astype(jnp.float32), axes=axes))(up[:, :, None, :], axes=(-2, -1))
        Yf = Uf * Kf[None, :, :, :]
        y = (lambda x, s, axes=(-2,-1): jnp.fft.irfft2(x, s=s, axes=axes).astype(jnp.bfloat16))(Yf, (1, L2), axes=(-2, -1))[:, :, 0, :L]
        y = (lambda x, *d: x.transpose(*d))(y, 0, 2, 1) + u * Dskip[None, None, :]
        return y

    x = A_x
    x = x + _A_ref(_layernorm(x, axis=-1), A_wqkv, A_w_phi, A_wo)
    x = x + _B_ref(_layernorm(x, axis=-1), B_A_re, B_A_im, B_B_re, B_B_im, B_C_re, B_C_im, B_log_dt, B_Dskip)
    x = x + _A_ref(_layernorm(x, axis=-1), A_wqkv, A_w_phi, A_wo)
    x = x + _B_ref(_layernorm(x, axis=-1), B_A_re, B_A_im, B_B_re, B_B_im, B_C_re, B_C_im, B_log_dt, B_Dskip)
    return x
```

```python
import functools
import math

import jax
import jax.numpy as jnp
import numpy as np
from jax import lax
import jax.experimental.pallas as pl
import jax.experimental.pallas.tpu as pltpu

S = 2048
D = 512
NS = 128
NA = 16
NK = 16
NFFT = 4096
LOG2E = 1.4426950408889634
F32 = jnp.float32
BF16 = jnp.bfloat16


def _np_constants():
    k1 = np.arange(NK)[:, None] + 0.5
    a = np.arange(NA)[None, :]
    ang = -2.0 * np.pi * k1 * a / 32.0
    f1 = np.concatenate([np.cos(ang), np.sin(ang)], axis=0)
    l1 = np.kron(f1, np.eye(8))
    l1inv = l1.T * (2.0 / NFFT)
    b = np.arange(128)[None, :, None]
    k2 = np.arange(128)[None, None, :]
    kk = (np.arange(NK)[:, None, None] + 0.5) + 32.0 * k2
    ang = -2.0 * np.pi * ((b * kk) % NFFT) / NFFT
    mr, mi = np.cos(ang), np.sin(ang)
    g = np.concatenate([np.concatenate([mr, mi], axis=2),
                        np.concatenate([-mi, mr], axis=2)], axis=1)
    sel = []
    for step in (2, 4, 8):
        m = np.zeros((128, 128), np.float32)
        for j in range(128):
            q, r = divmod(j, step)
            if r * 2 > step or (r * 2 == step and q % 2 == 1):
                q += 1
            src = q * step
            m[src if src < 128 else 1, j] = 1.0
        sel.append(m)
    sel = np.stack(sel, axis=0)
    e = np.zeros((128, 128), np.float32)
    for f in range(16):
        for h in range(8):
            e[f * 8 + h, f] = 1.0
    perm = np.zeros((128, 128), np.float32)
    for d in range(16):
        for h in range(8):
            perm[d * 8 + h, h * 16 + d] = 1.0
    l1inv = l1inv.reshape(128, 2, 128).transpose(1, 0, 2)
    g = g.reshape(NK, 4, 128, 128).transpose(0, 1, 2, 3)
    g = np.stack([np.stack([mr, mi], 1), np.stack([-mi, mr], 1)], 1)
    g = g.reshape(NK * 4, 128, 128)
    return (l1.astype(np.float32), l1inv.astype(np.float32), g.astype(np.float32),
            sel.astype(np.float32), e, perm)


_L1, _L1INV, _G, _SEL, _E, _PERM = _np_constants()


def _nt(a, b):
    return lax.dot_general(a, b, (((1,), (1,)), ((), ())), preferred_element_type=F32)


def _nn(a, b):
    return jnp.dot(a, b, preferred_element_type=F32)


def _cmul(ar, ai, br, bi):
    return ar * br - ai * bi, ar * bi + ai * br


def _layernorm_t(x):
    m = jnp.mean(x, axis=0, keepdims=True)
    xc = x - m
    v = jnp.mean(xc * xc, axis=0, keepdims=True)
    return xc * lax.rsqrt(v + 1e-5)


U_KGEN = 8
U_S1 = 4
U_LAST = 8
TS = 256
NP2 = 4
U_MID = 2
RC = 256


def _cat(xs, axis):
    return xs[0] if len(xs) == 1 else jnp.concatenate(xs, axis=axis)


def _kernel(x_ref, wqkv_ref, wphi_ref, wo_ref, are_ref, aim_ref, bre_ref, bim_ref,
            cre_ref, cim_ref, ldt_ref, dsk_ref, l1_ref, l1inv_ref, g_ref, sel_ref,
            e_ref, perm_ref, o_ref,
            xt, ut, ub, phiq, phik, vt, s1, s2, kf, kt, zr, zi, wt, wot, dskb, kvl):
    NT = S // TS
    NH = TS // 128
    sub8 = lax.broadcasted_iota(jnp.int32, (8, 128), 0)

    def gmat(k):
        return _cat([_cat([g_ref[k * 4 + 2 * i + o] for o in range(2)], 1) for i in range(2)], 0)

    row_h = lax.broadcasted_iota(jnp.int32, (128, 128), 0) % 8
    col_h16 = lax.broadcasted_iota(jnp.int32, (128, 128), 1) // 16
    col_h8 = lax.broadcasted_iota(jnp.int32, (128, 128), 1) % 8
    for g in range(4):
        m1 = wphi_ref[g * 128:(g + 1) * 128, :]
        pphi = _nt(e_ref[:, 0:16], m1)
        pphi = jnp.where(row_h == col_h16, pphi, 0.0).astype(BF16)
        for j in range(3):
            w = wqkv_ref[:, j * D + g * 128: j * D + (g + 1) * 128]
            r = _nt(pphi, w) * LOG2E if j < 2 else _nt(perm_ref[...], w)
            r = r.astype(BF16)
            for kk in range(4):
                wt[kk, g * 384 + j * 128: g * 384 + (j + 1) * 128, :] = r[:, kk * 128:(kk + 1) * 128]
        wo_p = _nn(perm_ref[...], wo_ref[g * 128:(g + 1) * 128, :])
        wot[g] = wo_p.T.astype(BF16)
    dskb[...] = jnp.broadcast_to(dsk_ref[...].astype(F32), (D, 128))

    dt = jnp.exp(ldt_ref[...].astype(F32)).astype(BF16).astype(F32)
    lr = dt * are_ref[...].astype(F32)
    li = dt * aim_ref[...].astype(F32)
    mag = jnp.exp(lr)
    pr, pi = mag * jnp.cos(li), mag * jnp.sin(li)
    for k in range(11):
        zr[k] = pr
        zi[k] = pi
        if k < 10:
            pr, pi = pr * pr - pi * pi, 2.0 * pr * pi
    wr, wi = _cmul(cre_ref[...].astype(F32), cim_ref[...].astype(F32),
                   dt * bre_ref[...].astype(F32), dt * bim_ref[...].astype(F32))
    zr[11] = wr
    zi[11] = wi

    lane16 = lax.broadcasted_iota(jnp.int32, (NA, 128), 1)
    row16 = lax.broadcasted_iota(jnp.int32, (NA, 128), 0)
    keep_lo = (lane16 < 64) & ~((lane16 == 1) & (row16 >= 2))

    def kgen_one(d):
        def bc(k):
            return (jnp.broadcast_to(zr[k, pl.ds(d, 1), :], (8, 128)),
                    jnp.broadcast_to(zi[k, pl.ds(d, 1), :], (8, 128)))

        def selbit(k, bit):
            r, i = bc(k)
            m = (sub8 & bit) != 0
            return jnp.where(m, r, 1.0), jnp.where(m, i, 0.0)
        yr, yi = selbit(0, 1)
        yr, yi = _cmul(yr, yi, *selbit(1, 2))
        yr, yi = _cmul(yr, yi, *selbit(2, 4))
        ys = [(yr, yi)]
        for k in (3, 4, 5):
            m = bc(k)
            ys = ys + [_cmul(a, b, *m) for a, b in ys]
        z64 = bc(6)
        ys = ys + [z64, z64]
        xr, xi = bc(11)
        xr, xi = _cmul(xr, xi, *selbit(7, 1))
        xr, xi = _cmul(xr, xi, *selbit(8, 2))
        xr, xi = _cmul(xr, xi, *selbit(9, 4))
        xs = [(xr, xi), _cmul(xr, xi, *bc(10))]
        xs = xs + [_cmul(a, b, *z64) for a, b in xs]
        ymat = _cat([_cat([a for a, _ in ys], 0), _cat([b for _, b in ys], 0)], 1).astype(BF16)
        xmat = _cat([_cat([a for a, _ in xs], 0), _cat([-b for _, b in xs], 0)], 1).astype(BF16)
        out = _nt(xmat, ymat)
        out = _cat([out, jnp.zeros((32, 48), F32)], 1)
        hi = pltpu.roll(out[16:32], 64, 1)
        kt[pl.ds(d, NA, stride=D), :] = jnp.where(keep_lo, out[0:16], hi)

    def kgen(i, carry):
        for j in range(U_KGEN):
            kgen_one(i * U_KGEN + j)
        return carry

    lax.fori_loop(0, D // U_KGEN, kgen, 0)

    for a in range(2, NA):
        c = 0 if a < 4 else (1 if a < 8 else 2)
        kt[a * D:(a + 1) * D, :] = _nn(kt[a * D:(a + 1) * D, :].astype(BF16), sel_ref[c])

    def stage1(load):
        def body(i, carry):
            for j in range(U_S1):
                base = (i * U_S1 + j) * 16
                outs = []
                for h in range(2):
                    r0 = pl.multiple_of(base + h * 8, 8)
                    rhs = _cat([load(r0, a) for a in range(NA)], 0).astype(BF16)
                    outs.append(_nn(l1_ref[...], rhs))
                r0 = pl.multiple_of(base, 16)
                for ri in range(2):
                    for k in range(NK):
                        q = (ri * NK + k) * 8
                        s1[k * 2 + ri, pl.ds(r0, 16), :] = _cat(
                            [outs[0][q:q + 8], outs[1][q:q + 8]], 0).astype(BF16)
            return carry
        lax.fori_loop(0, D // 16 // U_S1, body, 0)

    stage1(lambda r0, a: kt[pl.ds(a * D + r0, 8), :])

    def kf_body(k, carry):
        z = _nn(_cat([s1[2 * k], s1[2 * k + 1]], 1), gmat(k))
        kf[2 * k] = z[:, 0:128]
        kf[2 * k + 1] = z[:, 128:256]
        return carry
    lax.fori_loop(0, NK, kf_body, 0)

    def xin(i, carry):
        c0 = pl.multiple_of(i * TS, TS)
        xt[:, pl.ds(c0, TS)] = x_ref[pl.ds(c0, TS), :].astype(F32).T
        return carry
    lax.fori_loop(0, NT, xin, 0)

    def softmax_pair(p):
        ps = [p[f * 8:(f + 1) * 8] for f in range(16)]
        mx = functools.reduce(jnp.maximum, ps)
        mn = functools.reduce(jnp.minimum, ps)
        ep = [jnp.exp2(t - mx) for t in ps]
        en = [jnp.exp2(mn - t) for t in ps]
        rp = 1.0 / functools.reduce(jnp.add, ep)
        rn = 1.0 / functools.reduce(jnp.add, en)
        return _cat([t * rp for t in ep] + [t * rn for t in en], 0)

    def ln_to_ub(i, slot):
        c0 = pl.multiple_of(i * TS, TS)
        for h in range(NH):
            u = _layernorm_t(xt[:, pl.ds(c0 + h * 128, 128)]).astype(BF16)
            ub[slot * NH + h] = u

    def layer_a():
        ln_to_ub(0, 0)

        def p1(i, carry):
            slot = i % 2
            ln_to_ub(jnp.minimum(i + 1, NT - 1), 1 - slot)
            for g in range(4):
                w = _cat([wt[kk, g * 384:(g + 1) * 384, :] for kk in range(4)], 1)
                for h in range(NH):
                    p = _nn(w, ub[slot * NH + h])
                    t = i * NH + h
                    phiq[t, g * 256:(g + 1) * 256, :] = softmax_pair(p[0:128]).astype(BF16)
                    phik[t, g * 256:(g + 1) * 256, :] = softmax_pair(p[128:256]).astype(BF16)
                    vt[t, g * 128:(g + 1) * 128, :] = p[256:384].astype(BF16)
            return carry
        lax.fori_loop(0, NT, p1, 0)

        rowi = lax.broadcasted_iota(jnp.int32, (144, 256), 0)
        coli = lax.broadcasted_iota(jnp.int32, (144, 256), 1)
        kvmask = (rowi % 8 == coli % 8) & (rowi < 136)
        ones = jnp.ones((16, 512), BF16)

        def kv_body(g, carry):
            acc = None
            for c in range(S // 512):
                lhs = _cat([vt[c * 4 + j, pl.ds(pl.multiple_of(g * 128, 128), 128), :] for j in range(4)], 1)
                lhs = _cat([lhs, ones], 0)
                rhs = _cat([phik[c * 4 + j, pl.ds(pl.multiple_of(g * 256, 256), 256), :] for j in range(4)], 1)
                r = _nt(lhs, rhs)
                acc = r if acc is None else acc + r
            t = jnp.where(kvmask, acc, 0.0).astype(BF16)
            kvl[g * 2] = t[:, 0:128]
            kvl[g * 2 + 1] = t[:, 128:256]
            return carry
        lax.fori_loop(0, 4, kv_body, 0)

        def p2(i, carry):
            def num(h):
                os_ = []
                for g in range(4):
                    nd = _nn(_cat([kvl[g * 2], kvl[g * 2 + 1]], 1),
                             phiq[i * NP2 + h, g * 256:(g + 1) * 256, :])
                    r = 1.0 / (nd[128:136] + 1e-6)
                    os_ += [nd[d * 8:(d + 1) * 8] * r for d in range(16)]
                return _cat(os_, 0).astype(BF16)

            def fin(h, o):
                c0 = pl.multiple_of((i * NP2 + h) * 128, 128)
                w = _cat([wot[g] for g in range(4)], 1)
                xn = xt[:, pl.ds(c0, 128)] + _nn(w, o)
                xt[:, pl.ds(c0, 128)] = xn
                ut[:, pl.ds(c0, 128)] = _layernorm_t(xn)
            prev = num(0)
            for h in range(1, NP2):
                cur = num(h)
                fin(h - 1, prev)
                prev = cur
            fin(NP2 - 1, prev)
            return carry
        lax.fori_loop(0, S // 128 // NP2, p2, 0)

    def layer_b():
        stage1(lambda r0, a: ut[pl.ds(r0, 8), a * 128:(a + 1) * 128])

        def mid(i, carry):
            items = [(i * U_MID + kk, c) for kk in range(U_MID) for c in range(D // RC)]

            def fwd(k, c):
                rows = pl.ds(c * RC, RC)
                z = _nn(_cat([s1[2 * k, rows, :], s1[2 * k + 1, rows, :]], 1), gmat(k))
                yr, yi = _cmul(z[:, 0:128], z[:, 128:256], kf[2 * k, rows, :], kf[2 * k + 1, rows, :])
                return _cat([yr, yi], 1).astype(BF16)

            def inv(k, c, y):
                rows = pl.ds(c * RC, RC)
                v = _nt(y, gmat(k))
                s2[2 * k, rows, :] = v[:, 0:128]
                s2[2 * k + 1, rows, :] = v[:, 128:256]
            prev = fwd(*items[0])
            for n in range(1, len(items)):
                cur = fwd(*items[n])
                inv(*items[n - 1], prev)
                prev = cur
            inv(*items[-1], prev)
            return carry
        lax.fori_loop(0, NK // U_MID, mid, 0)

        def last(i, carry):
            for j in range(U_LAST):
                r0 = pl.multiple_of((i * U_LAST + j) * 8, 8)
                rhs = _cat([s2[2 * k + ri, pl.ds(r0, 8), :] for ri in range(2) for k in range(NK)],
                           0).astype(BF16)
                y = _nn(_cat([l1inv_ref[0], l1inv_ref[1]], 1), rhs)
                dk = dskb[pl.ds(r0, 8), :]
                for a in range(NA):
                    sl = (pl.ds(r0, 8), slice(a * 128, (a + 1) * 128))
                    xt[sl] = xt[sl] + (y[a * 8:(a + 1) * 8] + ut[sl] * dk)
            return carry
        lax.fori_loop(0, D // 8 // U_LAST, last, 0)

    def layers(i, carry):
        layer_a()
        layer_b()
        return carry
    lax.fori_loop(0, 2, layers, 0)

    def xout(i, carry):
        c0 = pl.multiple_of(i * TS, TS)
        o_ref[pl.ds(c0, TS), :] = xt[:, pl.ds(c0, TS)].T.astype(BF16)
        return carry
    lax.fori_loop(0, NT, xout, 0)


def _run(A_x, A_wqkv, A_w_phi, A_wo, B_A_re, B_A_im, B_B_re, B_B_im, B_C_re, B_C_im,
         B_log_dt, B_Dskip, interpret=False):
    consts = [jnp.asarray(c, dtype=BF16) for c in (_L1, _L1INV, _G, _SEL, _E, _PERM)]
    scratch = [
        pltpu.VMEM((D, S), F32),
        pltpu.VMEM((D, S), F32),
        pltpu.VMEM((2 * TS // 128, D, 128), BF16),
        pltpu.VMEM((S // 128, 2 * D, 128), BF16),
        pltpu.VMEM((S // 128, 2 * D, 128), BF16),
        pltpu.VMEM((S // 128, D, 128), BF16),
        pltpu.VMEM((NK * 2, D, 128), BF16),
        pltpu.VMEM((NK * 2, D, 128), F32),
        pltpu.VMEM((NK * 2, D, 128), F32),
        pltpu.VMEM((NA * D, 128), F32),
        pltpu.VMEM((12, D, NS), F32),
        pltpu.VMEM((12, D, NS), F32),
        pltpu.VMEM((4, 3 * D, 128), BF16),
        pltpu.VMEM((4, D, 128), BF16),
        pltpu.VMEM((D, 128), F32),
        pltpu.VMEM((8, 144, 128), BF16),
    ]
    out = pl.pallas_call(
        _kernel,
        out_shape=jax.ShapeDtypeStruct((S, D), BF16),
        scratch_shapes=scratch,
        compiler_params=pltpu.CompilerParams(vmem_limit_bytes=110 * 2**20),
        interpret=interpret,
        name="hedgehog_s4",
    )(A_x.reshape(S, D), A_wqkv, A_w_phi.reshape(D, 16), A_wo, B_A_re, B_A_im, B_B_re,
      B_B_im, B_C_re, B_C_im, B_log_dt.reshape(D, 1), B_Dskip.reshape(D, 1), *consts)
    return out.reshape(1, S, D)


@jax.jit
def pallas_interleave_layers__linear_kernel_hedgehog__ssm_conv_s4__prompt_kernel(
    A_x: jax.Array,
    A_wqkv: jax.Array,
    A_w_phi: jax.Array,
    A_wo: jax.Array,
    B_u: jax.Array,
    B_A_re: jax.Array,
    B_A_im: jax.Array,
    B_B_re: jax.Array,
    B_B_im: jax.Array,
    B_C_re: jax.Array,
    B_C_im: jax.Array,
    B_log_dt: jax.Array,
    B_Dskip: jax.Array,
):
    del B_u
    return _run(A_x, A_wqkv, A_w_phi, A_wo, B_A_re, B_A_im, B_B_re, B_B_im,
                B_C_re, B_C_im, B_log_dt, B_Dskip)
```

```python
import functools
import math

import jax
import jax.numpy as jnp
import numpy as np
from jax import lax
import jax.experimental.pallas as pl
import jax.experimental.pallas.tpu as pltpu

S = 2048
D = 512
NS = 128
NA = 16
NK = 16
NFFT = 4096
LOG2E = 1.4426950408889634
F32 = jnp.float32
BF16 = jnp.bfloat16


def _np_constants():
    k1 = np.arange(NK)[:, None] + 0.5
    a = np.arange(NA)[None, :]
    ang = -2.0 * np.pi * k1 * a / 32.0
    f1 = np.concatenate([np.cos(ang), np.sin(ang)], axis=0)
    l1 = np.kron(f1, np.eye(8))
    l1inv = l1.T * (2.0 / NFFT)
    b = np.arange(128)[None, :, None]
    k2 = np.arange(128)[None, None, :]
    kk = (np.arange(NK)[:, None, None] + 0.5) + 32.0 * k2
    ang = -2.0 * np.pi * ((b * kk) % NFFT) / NFFT
    mr, mi = np.cos(ang), np.sin(ang)
    g = np.concatenate([np.concatenate([mr, mi], axis=2),
                        np.concatenate([-mi, mr], axis=2)], axis=1)
    sel = []
    for step in (2, 4, 8):
        m = np.zeros((128, 128), np.float32)
        for j in range(128):
            q, r = divmod(j, step)
            if r * 2 > step or (r * 2 == step and q % 2 == 1):
                q += 1
            src = q * step
            m[src if src < 128 else 1, j] = 1.0
        sel.append(m)
    sel = np.stack(sel, axis=0)
    e = np.zeros((128, 128), np.float32)
    for f in range(16):
        for h in range(8):
            e[f * 8 + h, f] = 1.0
    perm = np.zeros((128, 128), np.float32)
    for d in range(16):
        for h in range(8):
            perm[d * 8 + h, h * 16 + d] = 1.0
    l1inv = l1inv.reshape(128, 2, 128).transpose(1, 0, 2)
    g = g.reshape(NK, 4, 128, 128).transpose(0, 1, 2, 3)
    g = np.stack([np.stack([mr, mi], 1), np.stack([-mi, mr], 1)], 1)
    g = g.reshape(NK * 4, 128, 128)
    return (l1.astype(np.float32), l1inv.astype(np.float32), g.astype(np.float32),
            sel.astype(np.float32), e, perm)


_L1, _L1INV, _G, _SEL, _E, _PERM = _np_constants()


def _nt(a, b):
    return lax.dot_general(a, b, (((1,), (1,)), ((), ())), preferred_element_type=F32)


def _nn(a, b):
    return jnp.dot(a, b, preferred_element_type=F32)


def _cmul(ar, ai, br, bi):
    return ar * br - ai * bi, ar * bi + ai * br


def _layernorm_t(x):
    m = jnp.mean(x, axis=0, keepdims=True)
    xc = x - m
    v = jnp.mean(xc * xc, axis=0, keepdims=True)
    return xc * lax.rsqrt(v + 1e-5)


FLAGS = {}
U_KGEN = 4
U_S1 = 4
U_LAST = 8
TS = 256
NP2 = 4
U_MID = 2
RC = 256


def _cat(xs, axis):
    return xs[0] if len(xs) == 1 else jnp.concatenate(xs, axis=axis)


def _kernel(x_hbm, wqkv_hbm, wphi_ref, wo_hbm, are_ref, aim_ref, bre_ref, bim_ref,
            cre_ref, cim_ref, ldt_ref, dsk_ref, l1_ref, l1inv_ref, g_hbm, sel_ref,
            e_ref, perm_ref, o_hbm,
            xt, ut, ub, phiq, phik, vt, s1, s2, kf, kt, zr, zi, wt, wot, dskb, kvl, kmat,
            x_ref, wqkv_ref, wo_ref, g_ref, o_ref, sems):
    NT = S // TS
    NH = TS // 128
    sub8 = lax.broadcasted_iota(jnp.int32, (8, 128), 0)
    cp_w = pltpu.make_async_copy(wqkv_hbm, wqkv_ref, sems.at[0])
    cp_wo = pltpu.make_async_copy(wo_hbm, wo_ref, sems.at[1])
    cp_x = pltpu.make_async_copy(x_hbm, x_ref, sems.at[2])
    cp_g = pltpu.make_async_copy(g_hbm, g_ref, sems.at[3])
    cp_w.start()
    cp_wo.start()
    cp_x.start()
    cp_g.start()

    def gmat(k):
        return _cat([_cat([g_ref[k * 4 + 2 * i + o] for o in range(2)], 1) for i in range(2)], 0)

    dskb[...] = jnp.broadcast_to(dsk_ref[...].astype(F32), (128, D)).T
    dt = jnp.exp(ldt_ref[...].astype(F32)).astype(BF16).astype(F32)
    dt = jnp.broadcast_to(dt, (128, D)).T
    lr = dt * are_ref[...].astype(F32)
    li = dt * aim_ref[...].astype(F32)
    mag = jnp.exp(lr)
    pr, pi = mag * jnp.cos(li), mag * jnp.sin(li)
    for k in range(11):
        zr[k] = pr
        zi[k] = pi
        if k < 10:
            pr, pi = pr * pr - pi * pi, 2.0 * pr * pi
    wr, wi = _cmul(cre_ref[...].astype(F32), cim_ref[...].astype(F32),
                   dt * bre_ref[...].astype(F32), dt * bim_ref[...].astype(F32))
    zr[11] = wr
    zi[11] = -wi

    row_h = lax.broadcasted_iota(jnp.int32, (128, 128), 0) % 8
    col_h16 = lax.broadcasted_iota(jnp.int32, (128, 128), 1) // 16
    col_h8 = lax.broadcasted_iota(jnp.int32, (128, 128), 1) % 8
    cp_w.wait()
    cp_wo.wait()
    wphi = wphi_ref[...].reshape(D, 16)
    for g in range(4):
        m1 = wphi[g * 128:(g + 1) * 128, :]
        pphi = _nt(e_ref[:, 0:16], m1)
        pphi = jnp.where(row_h == col_h16, pphi, 0.0).astype(BF16)
        for j in range(3):
            w = wqkv_ref[:, j * D + g * 128: j * D + (g + 1) * 128]
            r = _nt(pphi, w) * LOG2E if j < 2 else _nt(perm_ref[...], w)
            r = r.astype(BF16)
            for kk in range(4):
                wt[kk, g * 384 + j * 128: g * 384 + (j + 1) * 128, :] = r[:, kk * 128:(kk + 1) * 128]
        wo_p = _nn(perm_ref[...], wo_ref[g * 128:(g + 1) * 128, :])
        wot[g] = wo_p.T.astype(BF16)

    lane16 = lax.broadcasted_iota(jnp.int32, (NA, 128), 1)
    row16 = lax.broadcasted_iota(jnp.int32, (NA, 128), 0)
    keep_lo = (lane16 < 64) & ~((lane16 == 1) & (row16 >= 2))

    def kgen_one(d, slot):
        def bc(k):
            return (jnp.broadcast_to(zr[k, pl.ds(d, 1), :], (8, 128)),
                    jnp.broadcast_to(zi[k, pl.ds(d, 1), :], (8, 128)))

        def selbit(k, bit):
            r, i = bc(k)
            m = (sub8 & bit) != 0
            return jnp.where(m, r, 1.0), jnp.where(m, i, 0.0)

        def cmulc(ar, an, br, bi):
            return ar * br + an * bi, an * br - ar * bi
        yr, yi = selbit(0, 1)
        yr, yi = _cmul(yr, yi, *selbit(1, 2))
        yr, yi = _cmul(yr, yi, *selbit(2, 4))
        ys = [(yr, yi)]
        for k in (3, 4, 5):
            m = bc(k)
            ys = ys + [_cmul(a, b, *m) for a, b in ys]
        z64 = bc(6)
        ys = ys + [z64, z64]
        xr, xn = bc(11)
        xr, xn = cmulc(xr, xn, *selbit(7, 1))
        xr, xn = cmulc(xr, xn, *selbit(8, 2))
        xr, xn = cmulc(xr, xn, *selbit(9, 4))
        xs = [(xr, xn), cmulc(xr, xn, *bc(10))]
        xs = xs + [cmulc(a, b, *z64) for a, b in xs]
        kmat[slot * 2] = _cat([a for a, _ in ys] + [a for a, _ in xs], 0).astype(BF16)
        kmat[slot * 2 + 1] = _cat([b for _, b in ys] + [b for _, b in xs], 0).astype(BF16)

    def kgen_dot(slot):
        ymat = _cat([kmat[slot * 2, 0:80, :], kmat[slot * 2 + 1, 0:80, :]], 1)
        xmat = _cat([kmat[slot * 2, 80:112, :], kmat[slot * 2 + 1, 80:112, :]], 1)
        out = _nt(xmat, ymat)
        out = _cat([out, jnp.zeros((32, 48), F32)], 1)
        hi = pltpu.roll(out[16:32], 64, 1)
        return jnp.where(keep_lo, out[0:16], hi)

    def kgen_build(m, par):
        for j in range(U_KGEN):
            kgen_one(m * U_KGEN + j, par * U_KGEN + j)

    def kgen_dots(m, par):
        res = [kgen_dot(par * U_KGEN + j) for j in range(U_KGEN)]
        for j in range(U_KGEN):
            kt[pl.ds(m * U_KGEN + j, NA, stride=D), :] = res[j]

    kmat[...] = jnp.zeros(kmat.shape, BF16)

    def stage1(load):
        def body(i, carry):
            for j in range(U_S1):
                base = (i * U_S1 + j) * 16
                outs = []
                for h in range(2):
                    r0 = pl.multiple_of(base + h * 8, 8)
                    rhs = _cat([load(r0, a) for a in range(NA)], 0).astype(BF16)
                    outs.append(_nn(l1_ref[...], rhs))
                r0 = pl.multiple_of(base, 16)
                for ri in range(2):
                    for k in range(NK):
                        q = (ri * NK + k) * 8
                        s1[k * 2 + ri, pl.ds(r0, 16), :] = _cat(
                            [outs[0][q:q + 8], outs[1][q:q + 8]], 0).astype(BF16)
            return carry
        lax.fori_loop(0, D // 16 // U_S1, body, 0)

    def k_finish():
        cp_g.wait()
        kgen_dots(D // U_KGEN - 1, 1)
        for a in range(2, NA):
            c = 0 if a < 4 else (1 if a < 8 else 2)
            kt[a * D:(a + 1) * D, :] = _nn(kt[a * D:(a + 1) * D, :].astype(BF16), sel_ref[c])

        stage1(lambda r0, a: kt[pl.ds(a * D + r0, 8), :])

        def kf_body(k, carry):
            z = _nn(_cat([s1[2 * k], s1[2 * k + 1]], 1), gmat(k))
            kf[2 * k] = z[:, 0:128]
            kf[2 * k + 1] = z[:, 128:256]
            return carry
        lax.fori_loop(0, NK, kf_body, 0)

    cp_x.wait()

    def xin(i, carry):
        c0 = pl.multiple_of(i * TS, TS)
        xt[:, pl.ds(c0, TS)] = x_ref[pl.ds(c0, TS), :].astype(F32).T
        return carry
    lax.fori_loop(0, NT, xin, 0)

    def softmax_pair(p):
        ps = [p[f * 8:(f + 1) * 8] for f in range(16)]
        mx = functools.reduce(jnp.maximum, ps)
        mn = functools.reduce(jnp.minimum, ps)
        ep = [jnp.exp2(t - mx) for t in ps]
        en = [jnp.exp2(mn - t) for t in ps]
        rp = 1.0 / functools.reduce(jnp.add, ep)
        rn = 1.0 / functools.reduce(jnp.add, en)
        return _cat([t * rp for t in ep] + [t * rn for t in en], 0)

    def ln_to_ub(i, slot):
        c0 = pl.multiple_of(i * TS, TS)
        for h in range(NH):
            u = _layernorm_t(xt[:, pl.ds(c0 + h * 128, 128)]).astype(BF16)
            ub[slot * NH + h] = u

    def layer_a(with_kgen):
        ln_to_ub(0, 0)

        def p1(i, carry):
            slot = i % 2
            for g in range(4):
                if g == 2:
                    ln_to_ub(jnp.minimum(i + 1, NT - 1), 1 - slot)
                for h in range(NH):
                    n = g * NH + h
                    m = i * 4 * NH + n
                    t = i * NH + h

                    def proj(j):
                        r0 = g * 384 + j * 128
                        w = _cat([wt[kk, r0:r0 + 128, :] for kk in range(4)], 1)
                        return _nn(w, ub[slot * NH + h])

                    pq = proj(0)
                    pk = proj(1)
                    if with_kgen:
                        kgen_dots(jnp.maximum(m - 1, 0), (n + 1) % 2)
                    phiq[t, g * 256:(g + 1) * 256, :] = softmax_pair(pq).astype(BF16)
                    pv = proj(2)
                    if with_kgen:
                        kgen_build(m, n % 2)
                    phik[t, g * 256:(g + 1) * 256, :] = softmax_pair(pk).astype(BF16)
                    vt[t, g * 128:(g + 1) * 128, :] = pv.astype(BF16)
            return carry
        lax.fori_loop(0, NT, p1, 0)

        rowi = lax.broadcasted_iota(jnp.int32, (144, 256), 0)
        coli = lax.broadcasted_iota(jnp.int32, (144, 256), 1)
        kvmask = (rowi % 8 == coli % 8) & (rowi < 136)
        ones = jnp.ones((16, 512), BF16)

        def kv_body(g, carry):
            acc = None
            for c in range(S // 512):
                lhs = _cat([vt[c * 4 + j, pl.ds(pl.multiple_of(g * 128, 128), 128), :] for j in range(4)], 1)
                lhs = _cat([lhs, ones], 0)
                rhs = _cat([phik[c * 4 + j, pl.ds(pl.multiple_of(g * 256, 256), 256), :] for j in range(4)], 1)
                r = _nt(lhs, rhs)
                acc = r if acc is None else acc + r
            t = jnp.where(kvmask, acc, 0.0).astype(BF16)
            kvl[g * 2] = t[:, 0:128]
            kvl[g * 2 + 1] = t[:, 128:256]
            return carry
        lax.fori_loop(0, 4, kv_body, 0)

        def p2(i, carry, with_kgen=with_kgen):
            def num(h):
                os_ = []
                for g in range(4):
                    nd = _nn(_cat([kvl[g * 2], kvl[g * 2 + 1]], 1),
                             phiq[i * NP2 + h, g * 256:(g + 1) * 256, :])
                    r = 1.0 / (nd[128:136] + 1e-6)
                    os_ += [nd[d * 8:(d + 1) * 8] * r for d in range(16)]
                return _cat(os_, 0).astype(BF16)

            def fin(h, o):
                c0 = pl.multiple_of((i * NP2 + h) * 128, 128)
                w = _cat([wot[g] for g in range(4)], 1)
                xn = xt[:, pl.ds(c0, 128)] + _nn(w, o)
                xt[:, pl.ds(c0, 128)] = xn
                ut[:, pl.ds(c0, 128)] = _layernorm_t(xn)

            def kg(h):
                if with_kgen:
                    for q in range(4):
                        n = h * 4 + q
                        m = 64 + i * NP2 * 4 + n
                        kgen_dots(m - 1, (n + 1) % 2)
                        kgen_build(m, n % 2)
            prev = num(0)
            kg(0)
            for h in range(1, NP2):
                cur = num(h)
                fin(h - 1, prev)
                kg(h)
                prev = cur
            fin(NP2 - 1, prev)
            return carry
        lax.fori_loop(0, S // 128 // NP2, p2, 0)

    def layer_b():
        stage1(lambda r0, a: ut[pl.ds(r0, 8), a * 128:(a + 1) * 128])

        def mid(i, carry):
            items = [(i * U_MID + kk, c) for kk in range(U_MID) for c in range(D // RC)]

            def fwd(k, c):
                rows = pl.ds(c * RC, RC)
                z = _nn(_cat([s1[2 * k, rows, :], s1[2 * k + 1, rows, :]], 1), gmat(k))
                yr, yi = _cmul(z[:, 0:128], z[:, 128:256], kf[2 * k, rows, :], kf[2 * k + 1, rows, :])
                return _cat([yr, yi], 1).astype(BF16)

            def inv(k, c, y):
                rows = pl.ds(c * RC, RC)
                v = _nt(y, gmat(k))
                s2[2 * k, rows, :] = v[:, 0:128]
                s2[2 * k + 1, rows, :] = v[:, 128:256]
            prev = fwd(*items[0])
            for n in range(1, len(items)):
                cur = fwd(*items[n])
                inv(*items[n - 1], prev)
                prev = cur
            inv(*items[-1], prev)
            return carry
        lax.fori_loop(0, NK // U_MID, mid, 0)

        def last(i, carry):
            for j in range(U_LAST):
                r0 = pl.multiple_of((i * U_LAST + j) * 8, 8)
                rhs = _cat([s2[2 * k + ri, pl.ds(r0, 8), :] for ri in range(2) for k in range(NK)],
                           0).astype(BF16)
                y = _nn(_cat([l1inv_ref[0], l1inv_ref[1]], 1), rhs)
                dk = dskb[pl.ds(r0, 8), :]
                for a in range(NA):
                    sl = (pl.ds(r0, 8), slice(a * 128, (a + 1) * 128))
                    xt[sl] = xt[sl] + (y[a * 8:(a + 1) * 8] + ut[sl] * dk)
            return carry
        lax.fori_loop(0, D // 8 // U_LAST, last, 0)

    layer_a(True)
    k_finish()
    layer_b()
    layer_a(False)
    layer_b()

    def xout(i, carry):
        c0 = pl.multiple_of(i * TS, TS)
        o_ref[pl.ds(c0, TS), :] = xt[:, pl.ds(c0, TS)].T.astype(BF16)
        pltpu.make_async_copy(o_ref.at[pl.ds(c0, TS), :], o_hbm.at[pl.ds(c0, TS), :],
                              sems.at[4 + i]).start()
        return carry
    lax.fori_loop(0, NT, xout, 0)
    for i in range(NT):
        pltpu.make_async_copy(o_ref.at[pl.ds(i * TS, TS), :], o_hbm.at[pl.ds(i * TS, TS), :],
                              sems.at[4 + i]).wait()


def _run(A_x, A_wqkv, A_w_phi, A_wo, B_A_re, B_A_im, B_B_re, B_B_im, B_C_re, B_C_im,
         B_log_dt, B_Dskip, interpret=False):
    consts = [jnp.asarray(c, dtype=BF16) for c in (_L1, _L1INV, _G, _SEL, _E, _PERM)]
    scratch = [
        pltpu.VMEM((D, S), F32),
        pltpu.VMEM((D, S), F32),
        pltpu.VMEM((2 * TS // 128, D, 128), BF16),
        pltpu.VMEM((S // 128, 2 * D, 128), BF16),
        pltpu.VMEM((S // 128, 2 * D, 128), BF16),
        pltpu.VMEM((S // 128, D, 128), BF16),
        pltpu.VMEM((NK * 2, D, 128), BF16),
        pltpu.VMEM((NK * 2, D, 128), F32),
        pltpu.VMEM((NK * 2, D, 128), F32),
        pltpu.VMEM((NA * D, 128), F32),
        pltpu.VMEM((12, D, NS), F32),
        pltpu.VMEM((12, D, NS), F32),
        pltpu.VMEM((4, 3 * D, 128), BF16),
        pltpu.VMEM((4, D, 128), BF16),
        pltpu.VMEM((D, 128), F32),
        pltpu.VMEM((8, 144, 128), BF16),
        pltpu.VMEM((4 * U_KGEN, 112, 128), BF16),
        pltpu.VMEM((S, D), BF16),
        pltpu.VMEM((D, 3 * D), BF16),
        pltpu.VMEM((D, D), BF16),
        pltpu.VMEM((NK * 4, 128, 128), BF16),
        pltpu.VMEM((S, D), BF16),
        pltpu.SemaphoreType.DMA((4 + S // TS,)),
    ]
    out = pl.pallas_call(
        _kernel,
        out_shape=jax.ShapeDtypeStruct((S, D), BF16),
        in_specs=[pl.BlockSpec(memory_space=pl.ANY) if i in (0, 1, 3, 14)
                  else pl.BlockSpec(memory_space=pltpu.VMEM) for i in range(18)],
        out_specs=pl.BlockSpec(memory_space=pl.ANY),
        scratch_shapes=scratch,
        compiler_params=pltpu.CompilerParams(vmem_limit_bytes=110 * 2**20, flags=FLAGS),
        interpret=interpret,
        name="hedgehog_s4",
    )(A_x.reshape(S, D), A_wqkv, A_w_phi, A_wo, B_A_re, B_A_im, B_B_re,
      B_B_im, B_C_re, B_C_im, B_log_dt.reshape(1, D), B_Dskip.reshape(1, D), *consts)
    return out.reshape(1, S, D)


@jax.jit
def pallas_interleave_layers__linear_kernel_hedgehog__ssm_conv_s4__prompt_kernel(
    A_x: jax.Array,
    A_wqkv: jax.Array,
    A_w_phi: jax.Array,
    A_wo: jax.Array,
    B_u: jax.Array,
    B_A_re: jax.Array,
    B_A_im: jax.Array,
    B_B_re: jax.Array,
    B_B_im: jax.Array,
    B_C_re: jax.Array,
    B_C_im: jax.Array,
    B_log_dt: jax.Array,
    B_Dskip: jax.Array,
):
    del B_u
    return _run(A_x, A_wqkv, A_w_phi, A_wo, B_A_re, B_A_im, B_B_re, B_B_im,
                B_C_re, B_C_im, B_log_dt, B_Dskip)
```

```python
import functools
import math

import jax
import jax.numpy as jnp
import numpy as np
from jax import lax
import jax.experimental.pallas as pl
import jax.experimental.pallas.tpu as pltpu

S = 2048
D = 512
NS = 128
NA = 16
NK = 16
NFFT = 4096
LOG2E = 1.4426950408889634
F32 = jnp.float32
BF16 = jnp.bfloat16


def _np_constants():
    k1 = np.arange(NK)[:, None] + 0.5
    a = np.arange(NA)[None, :]
    ang = -2.0 * np.pi * k1 * a / 32.0
    f1 = np.concatenate([np.cos(ang), np.sin(ang)], axis=0)
    l1 = np.kron(f1, np.eye(8))
    l1inv = l1.T * (2.0 / NFFT)
    b = np.arange(128)[None, :, None]
    k2 = np.arange(128)[None, None, :]
    kk = (np.arange(NK)[:, None, None] + 0.5) + 32.0 * k2
    ang = -2.0 * np.pi * ((b * kk) % NFFT) / NFFT
    mr, mi = np.cos(ang), np.sin(ang)
    g = np.concatenate([np.concatenate([mr, mi], axis=2),
                        np.concatenate([-mi, mr], axis=2)], axis=1)
    sel = []
    for step in (2, 4, 8):
        m = np.zeros((128, 128), np.float32)
        for j in range(128):
            q, r = divmod(j, step)
            if r * 2 > step or (r * 2 == step and q % 2 == 1):
                q += 1
            src = q * step
            m[src if src < 128 else 1, j] = 1.0
        sel.append(m)
    sel = np.stack(sel, axis=0)
    e = np.zeros((128, 128), np.float32)
    for f in range(16):
        for h in range(8):
            e[f * 8 + h, f] = 1.0
    perm = np.zeros((128, 128), np.float32)
    for d in range(16):
        for h in range(8):
            perm[d * 8 + h, h * 16 + d] = 1.0
    l1inv = l1inv.reshape(128, 2, 128).transpose(1, 0, 2)
    g = np.stack([mr, mi - mr, mr + mi], 1).reshape(NK * 3, 128, 128)
    return (l1.astype(np.float32), l1inv.astype(np.float32), g.astype(np.float32),
            sel.astype(np.float32), e, perm)


_L1, _L1INV, _G, _SEL, _E, _PERM = _np_constants()


def _nt(a, b):
    return lax.dot_general(a, b, (((1,), (1,)), ((), ())), preferred_element_type=F32)


def _nn(a, b):
    return jnp.dot(a, b, preferred_element_type=F32)


def _cmul(ar, ai, br, bi):
    return ar * br - ai * bi, ar * bi + ai * br


def _layernorm_t(x):
    m = jnp.mean(x, axis=0, keepdims=True)
    xc = x - m
    v = jnp.mean(xc * xc, axis=0, keepdims=True)
    return xc * lax.rsqrt(v + 1e-5)


FLAGS = {}
U_KGEN = 4
KSPLIT = (8, 8, 8, 8)
KRING = 8
KLAG = 4
U_S1 = 8
U_LAST = 16
TS = 512
U_MID = 4
RC = 256


def _cat(xs, axis):
    return xs[0] if len(xs) == 1 else jnp.concatenate(xs, axis=axis)


def _kernel(x_hbm, wqkv_hbm, wphi_ref, wo_hbm, are_ref, aim_ref, bre_ref, bim_ref,
            cre_ref, cim_ref, ldt_ref, dsk_ref, l1_ref, l1inv_ref, g_hbm, sel_ref,
            e_ref, perm_ref, o_hbm,
            xt, ut, ub, phiq, phik, vt, s1, s1k, s2, kf, kt, zr, zi, wt, wot, dskb, kvl, kmat,
            x_ref, wqkv_ref, wo_ref, g_ref, o_ref, sems):
    NT = S // TS
    NH = TS // 128
    sub8 = lax.broadcasted_iota(jnp.int32, (8, 128), 0)
    cp_w = pltpu.make_async_copy(wqkv_hbm, wqkv_ref, sems.at[0])
    cp_wo = pltpu.make_async_copy(wo_hbm, wo_ref, sems.at[1])
    cp_x = pltpu.make_async_copy(x_hbm, x_ref, sems.at[2])
    cp_g = pltpu.make_async_copy(g_hbm, g_ref, sems.at[3])
    cp_w.start()
    cp_wo.start()
    cp_x.start()
    cp_g.start()

    def dft_fwd(src, k, rows):
        k1 = _nn(src[3 * k + 2, rows, :], g_ref[3 * k])
        k2 = _nn(src[3 * k, rows, :], g_ref[3 * k + 1])
        k3 = _nn(src[3 * k + 1, rows, :], g_ref[3 * k + 2])
        return k1 - k3, k1 + k2

    dskb[...] = jnp.broadcast_to(dsk_ref[...].astype(F32), (128, D)).T
    dt = jnp.exp(ldt_ref[...].astype(F32)).astype(BF16).astype(F32)
    dt = jnp.broadcast_to(dt, (128, D)).T
    lr = dt * are_ref[...].astype(F32)
    li = dt * aim_ref[...].astype(F32)
    mag = jnp.exp(lr)
    pr, pi = mag * jnp.cos(li), mag * jnp.sin(li)
    for k in range(11):
        zr[k] = pr
        zi[k] = pi
        if k < 10:
            pr, pi = pr * pr - pi * pi, 2.0 * pr * pi
    wr, wi = _cmul(cre_ref[...].astype(F32), cim_ref[...].astype(F32),
                   dt * bre_ref[...].astype(F32), dt * bim_ref[...].astype(F32))
    zr[11] = wr
    zi[11] = -wi

    row_h = lax.broadcasted_iota(jnp.int32, (128, 128), 0) % 8
    col_h16 = lax.broadcasted_iota(jnp.int32, (128, 128), 1) // 16
    col_h8 = lax.broadcasted_iota(jnp.int32, (128, 128), 1) % 8
    cp_w.wait()
    cp_wo.wait()
    wphi = wphi_ref[...].reshape(D, 16)
    for g in range(4):
        m1 = wphi[g * 128:(g + 1) * 128, :]
        pphi = _nt(e_ref[:, 0:16], m1)
        pphi = jnp.where(row_h == col_h16, pphi, 0.0).astype(BF16)
        for j in range(3):
            w = wqkv_ref[:, j * D + g * 128: j * D + (g + 1) * 128]
            r = _nt(pphi, w) * LOG2E if j < 2 else _nt(perm_ref[...], w)
            r = r.astype(BF16)
            for kk in range(4):
                wt[kk, g * 384 + j * 128: g * 384 + (j + 1) * 128, :] = r[:, kk * 128:(kk + 1) * 128]
        wo_p = _nn(perm_ref[...], wo_ref[g * 128:(g + 1) * 128, :])
        wot[g] = wo_p.T.astype(BF16)

    lane16 = lax.broadcasted_iota(jnp.int32, (NA, 128), 1)
    row16 = lax.broadcasted_iota(jnp.int32, (NA, 128), 0)
    keep_lo = (lane16 < 64) & ~((lane16 == 1) & (row16 >= 2))

    def kgen_one(d, slot):
        def bc(k):
            return (jnp.broadcast_to(zr[k, pl.ds(d, 1), :], (8, 128)),
                    jnp.broadcast_to(zi[k, pl.ds(d, 1), :], (8, 128)))

        def selbit(k, bit):
            r, i = bc(k)
            m = (sub8 & bit) != 0
            return jnp.where(m, r, 1.0), jnp.where(m, i, 0.0)

        def cmulc(ar, an, br, bi):
            return ar * br + an * bi, an * br - ar * bi
        yr, yi = selbit(0, 1)
        yr, yi = _cmul(yr, yi, *selbit(1, 2))
        yr, yi = _cmul(yr, yi, *selbit(2, 4))
        ys = [(yr, yi)]
        for k in (3, 4, 5):
            m = bc(k)
            ys = ys + [_cmul(a, b, *m) for a, b in ys]
        z64 = bc(6)
        ys = ys + [z64, z64]
        xr, xn = bc(11)
        xr, xn = cmulc(xr, xn, *selbit(7, 1))
        xr, xn = cmulc(xr, xn, *selbit(8, 2))
        xr, xn = cmulc(xr, xn, *selbit(9, 4))
        xs = [(xr, xn), cmulc(xr, xn, *bc(10))]
        xs = xs + [cmulc(a, b, *z64) for a, b in xs]
        kmat[slot * 2] = _cat([a for a, _ in ys] + [a for a, _ in xs], 0).astype(BF16)
        kmat[slot * 2 + 1] = _cat([b for _, b in ys] + [b for _, b in xs], 0).astype(BF16)

    def kgen_dot(slot):
        ymat = _cat([kmat[slot * 2, 0:80, :], kmat[slot * 2 + 1, 0:80, :]], 1)
        xmat = _cat([kmat[slot * 2, 80:112, :], kmat[slot * 2 + 1, 80:112, :]], 1)
        out = _nt(xmat, ymat)
        out = _cat([out, jnp.zeros((32, 48), F32)], 1)
        hi = pltpu.roll(out[16:32], 64, 1)
        return jnp.where(keep_lo, out[0:16], hi)

    def kgen_build(m, par):
        for j in range(U_KGEN):
            kgen_one(m * U_KGEN + j, par * U_KGEN + j)

    def kgen_dots(m, par):
        res = [kgen_dot(par * U_KGEN + j) for j in range(U_KGEN)]
        for j in range(U_KGEN):
            kt[pl.ds(m * U_KGEN + j, NA, stride=D), :] = res[j]

    class Ticker:
        def __init__(self, base, nstep, npts):
            self.ops = []
            for n in range(nstep):
                m = base + n
                for j in range(U_KGEN):
                    self.ops.append(functools.partial(
                        kgen_dot_store, jnp.maximum(m - KLAG, 0) * U_KGEN + j,
                        ((n - KLAG) % KRING) * U_KGEN + j))
                    self.ops.append(functools.partial(
                        kgen_one, m * U_KGEN + j, (n % KRING) * U_KGEN + j))
            self.npts, self.i, self.done = npts, 0, 0

        def __call__(self):
            self.i += 1
            tgt = len(self.ops) * self.i // self.npts
            for op in self.ops[self.done:tgt]:
                op()
            self.done = tgt

    def kgen_dot_store(d, slot):
        kt[pl.ds(d, NA, stride=D), :] = kgen_dot(slot)

    def no_tick():
        pass

    KP1, KKV, KP2, KS1 = KSPLIT
    assert 4 * (KP1 + KKV + KP2 + KS1) * U_KGEN == D
    kmat[...] = jnp.zeros(kmat.shape, BF16)

    def stage1(load, dst, hook=None):
        def body(i, carry):
            tick = hook(i) if hook is not None else no_tick
            for j in range(U_S1):
                base = (i * U_S1 + j) * 16
                outs = []
                for h in range(2):
                    r0 = pl.multiple_of(base + h * 8, 8)
                    rhs = _cat([load(r0, a) for a in range(NA)], 0).astype(BF16)
                    outs.append(_nn(l1_ref[...], rhs))
                    tick()
                r0 = pl.multiple_of(base, 16)
                for k in range(NK):
                    re = _cat([o[k * 8:k * 8 + 8] for o in outs], 0)
                    im = _cat([o[128 + k * 8:128 + k * 8 + 8] for o in outs], 0)
                    dst[k * 3, pl.ds(r0, 16), :] = re.astype(BF16)
                    dst[k * 3 + 1, pl.ds(r0, 16), :] = im.astype(BF16)
                    dst[k * 3 + 2, pl.ds(r0, 16), :] = (re + im).astype(BF16)
            return carry
        lax.fori_loop(0, D // 16 // U_S1, body, 0)

    def k_finish():
        cp_g.wait()
        for q in range(KLAG, 0, -1):
            kgen_dots(D // U_KGEN - q, (-q) % KRING)
        for a in range(2, NA):
            c = 0 if a < 4 else (1 if a < 8 else 2)
            kt[a * D:(a + 1) * D, :] = _nn(kt[a * D:(a + 1) * D, :].astype(BF16), sel_ref[c])

        stage1(lambda r0, a: kt[pl.ds(a * D + r0, 8), :], s1k)

        def kf_body(i, carry):
            for kk in range(2):
                k = i * 2 + kk
                kf[2 * k], kf[2 * k + 1] = dft_fwd(s1k, k, slice(None))
            return carry
        lax.fori_loop(0, NK // 2, kf_body, 0)

    cp_x.wait()

    def xin(i, carry):
        c0 = pl.multiple_of(i * TS, TS)
        xt[:, pl.ds(c0, TS)] = x_ref[pl.ds(c0, TS), :].astype(F32).T
        return carry
    lax.fori_loop(0, NT, xin, 0)

    def softmax_pair(p):
        ps = [p[f * 8:(f + 1) * 8] for f in range(16)]
        mx = functools.reduce(jnp.maximum, ps)
        mn = functools.reduce(jnp.minimum, ps)
        ep = [jnp.exp2(t - mx) for t in ps]
        en = [jnp.exp2(mn - t) for t in ps]
        rp = 1.0 / functools.reduce(jnp.add, ep)
        rn = 1.0 / functools.reduce(jnp.add, en)
        return _cat([t * rp for t in ep] + [t * rn for t in en], 0)

    def ln_to_ub(i, slot):
        c0 = pl.multiple_of(i * TS, TS)
        for h in range(NH):
            u = _layernorm_t(xt[:, pl.ds(c0 + h * 128, 128)]).astype(BF16)
            ub[slot * NH + h] = u

    def layer_a(with_kgen):
        ln_to_ub(0, 0)

        def p1(i, carry):
            slot = i % 2
            tick = Ticker(i * KP1, KP1, 48) if with_kgen else no_tick
            for g in range(4):
                if g == 2:
                    ln_to_ub(jnp.minimum(i + 1, NT - 1), 1 - slot)
                for h in range(NH):
                    n = g * NH + h
                    t = i * NH + h

                    def proj(j):
                        r0 = g * 384 + j * 128
                        w = _cat([wt[kk, r0:r0 + 128, :] for kk in range(4)], 1)
                        return _nn(w, ub[slot * NH + h])

                    pq = proj(0)
                    tick()
                    pk = proj(1)
                    tick()
                    phiq[t, g * 256:(g + 1) * 256, :] = softmax_pair(pq).astype(BF16)
                    pv = proj(2)
                    tick()
                    phik[t, g * 256:(g + 1) * 256, :] = softmax_pair(pk).astype(BF16)
                    vt[t, g * 128:(g + 1) * 128, :] = pv.astype(BF16)
            return carry
        lax.fori_loop(0, NT, p1, 0)

        rowi = lax.broadcasted_iota(jnp.int32, (144, 256), 0)
        coli = lax.broadcasted_iota(jnp.int32, (144, 256), 1)
        kvmask = (rowi % 8 == coli % 8) & (rowi < 136)
        ones = jnp.ones((16, 128), BF16)

        def kv_body(g, carry):
            tick = Ticker(4 * KP1 + g * KKV, KKV, 16) if with_kgen else no_tick
            acc = None
            for c in range(S // 128):
                lhs = _cat([vt[c, pl.ds(pl.multiple_of(g * 128, 128), 128), :], ones], 0)
                r = _nt(lhs, phik[c, pl.ds(pl.multiple_of(g * 256, 256), 256), :])
                acc = r if acc is None else acc + r
                tick()
            t = jnp.where(kvmask, acc, 0.0).astype(BF16)
            kvl[g * 2] = t[:, 0:128]
            kvl[g * 2 + 1] = t[:, 128:256]
            return carry
        lax.fori_loop(0, 4, kv_body, 0)

        NP2 = 4 if with_kgen else 8

        def p2(i, carry):
            tick = Ticker(4 * (KP1 + KKV) + i * KP2, KP2, 5 * NP2) if with_kgen else no_tick

            def num(h):
                os_ = []
                for g in range(4):
                    nd = _nn(_cat([kvl[g * 2], kvl[g * 2 + 1]], 1),
                             phiq[i * NP2 + h, g * 256:(g + 1) * 256, :])
                    r = 1.0 / (nd[128:136] + 1e-6)
                    os_ += [nd[d * 8:(d + 1) * 8] * r for d in range(16)]
                    tick()
                return _cat(os_, 0).astype(BF16)

            def fin(h, o):
                c0 = pl.multiple_of((i * NP2 + h) * 128, 128)
                w = _cat([wot[g] for g in range(4)], 1)
                xn = xt[:, pl.ds(c0, 128)] + _nn(w, o)
                xt[:, pl.ds(c0, 128)] = xn
                ut[:, pl.ds(c0, 128)] = _layernorm_t(xn)
                tick()

            prev = num(0)
            for h in range(1, NP2):
                cur = num(h)
                fin(h - 1, prev)
                prev = cur
            fin(NP2 - 1, prev)
            return carry
        lax.fori_loop(0, S // 128 // NP2, p2, 0)

    def layer_b(first):
        def hook(i):
            return Ticker(4 * (KP1 + KKV + KP2) + i * KS1, KS1, 2 * U_S1)
        stage1(lambda r0, a: ut[pl.ds(r0, 8), a * 128:(a + 1) * 128], s1, hook if first else None)
        if first:
            k_finish()

        def mid(i, carry):
            items = [(i * U_MID + kk, c) for kk in range(U_MID) for c in range(D // RC)]

            def fwd(k, c):
                rows = pl.ds(c * RC, RC)
                zr_, zi_ = dft_fwd(s1, k, rows)
                yr, yi = _cmul(zr_, zi_, kf[2 * k, rows, :], kf[2 * k + 1, rows, :])
                return yr.astype(BF16), yi.astype(BF16), (yr + yi).astype(BF16)

            def inv(k, c, y):
                rows = pl.ds(c * RC, RC)
                j1 = _nt(y[2], g_ref[3 * k])
                s2[2 * k, rows, :] = j1 + _nt(y[1], g_ref[3 * k + 1])
                s2[2 * k + 1, rows, :] = j1 - _nt(y[0], g_ref[3 * k + 2])
            prev = fwd(*items[0])
            for n in range(1, len(items)):
                cur = fwd(*items[n])
                inv(*items[n - 1], prev)
                prev = cur
            inv(*items[-1], prev)
            return carry
        lax.fori_loop(0, NK // U_MID, mid, 0)

        def last(i, carry):
            for j in range(U_LAST):
                r0 = pl.multiple_of((i * U_LAST + j) * 8, 8)
                rhs = _cat([s2[2 * k + ri, pl.ds(r0, 8), :] for ri in range(2) for k in range(NK)],
                           0).astype(BF16)
                y = _nn(_cat([l1inv_ref[0], l1inv_ref[1]], 1), rhs)
                dk = dskb[pl.ds(r0, 8), :]
                for a in range(NA):
                    sl = (pl.ds(r0, 8), slice(a * 128, (a + 1) * 128))
                    xt[sl] = xt[sl] + (y[a * 8:(a + 1) * 8] + ut[sl] * dk)
            return carry
        lax.fori_loop(0, D // 8 // U_LAST, last, 0)

    layer_a(True)
    layer_b(True)
    layer_a(False)
    layer_b(False)

    def xout(i, carry):
        c0 = pl.multiple_of(i * TS, TS)
        o_ref[pl.ds(c0, TS), :] = xt[:, pl.ds(c0, TS)].T.astype(BF16)
        pltpu.make_async_copy(o_ref.at[pl.ds(c0, TS), :], o_hbm.at[pl.ds(c0, TS), :],
                              sems.at[4 + i]).start()
        return carry
    lax.fori_loop(0, NT, xout, 0)
    for i in range(NT):
        pltpu.make_async_copy(o_ref.at[pl.ds(i * TS, TS), :], o_hbm.at[pl.ds(i * TS, TS), :],
                              sems.at[4 + i]).wait()


def _run(A_x, A_wqkv, A_w_phi, A_wo, B_A_re, B_A_im, B_B_re, B_B_im, B_C_re, B_C_im,
         B_log_dt, B_Dskip, interpret=False):
    consts = [jnp.asarray(c, dtype=BF16) for c in (_L1, _L1INV, _G, _SEL, _E, _PERM)]
    scratch = [
        pltpu.VMEM((D, S), F32),
        pltpu.VMEM((D, S), F32),
        pltpu.VMEM((2 * TS // 128, D, 128), BF16),
        pltpu.VMEM((S // 128, 2 * D, 128), BF16),
        pltpu.VMEM((S // 128, 2 * D, 128), BF16),
        pltpu.VMEM((S // 128, D, 128), BF16),
        pltpu.VMEM((NK * 3, D, 128), BF16),
        pltpu.VMEM((NK * 3, D, 128), BF16),
        pltpu.VMEM((NK * 2, D, 128), F32),
        pltpu.VMEM((NK * 2, D, 128), F32),
        pltpu.VMEM((NA * D, 128), F32),
        pltpu.VMEM((12, D, NS), F32),
        pltpu.VMEM((12, D, NS), F32),
        pltpu.VMEM((4, 3 * D, 128), BF16),
        pltpu.VMEM((4, D, 128), BF16),
        pltpu.VMEM((D, 128), F32),
        pltpu.VMEM((8, 144, 128), BF16),
        pltpu.VMEM((2 * KRING * U_KGEN, 112, 128), BF16),
        pltpu.VMEM((S, D), BF16),
        pltpu.VMEM((D, 3 * D), BF16),
        pltpu.VMEM((D, D), BF16),
        pltpu.VMEM((NK * 3, 128, 128), BF16),
        pltpu.VMEM((S, D), BF16),
        pltpu.SemaphoreType.DMA((4 + S // TS,)),
    ]
    out = pl.pallas_call(
        _kernel,
        out_shape=jax.ShapeDtypeStruct((S, D), BF16),
        in_specs=[pl.BlockSpec(memory_space=pl.ANY) if i in (0, 1, 3, 14)
                  else pl.BlockSpec(memory_space=pltpu.VMEM) for i in range(18)],
        out_specs=pl.BlockSpec(memory_space=pl.ANY),
        scratch_shapes=scratch,
        compiler_params=pltpu.CompilerParams(vmem_limit_bytes=110 * 2**20, flags=FLAGS),
        interpret=interpret,
        name="hedgehog_s4",
    )(A_x.reshape(S, D), A_wqkv, A_w_phi, A_wo, B_A_re, B_A_im, B_B_re,
      B_B_im, B_C_re, B_C_im, B_log_dt.reshape(1, D), B_Dskip.reshape(1, D), *consts)
    return out.reshape(1, S, D)


@jax.jit
def pallas_interleave_layers__linear_kernel_hedgehog__ssm_conv_s4__prompt_kernel(
    A_x: jax.Array,
    A_wqkv: jax.Array,
    A_w_phi: jax.Array,
    A_wo: jax.Array,
    B_u: jax.Array,
    B_A_re: jax.Array,
    B_A_im: jax.Array,
    B_B_re: jax.Array,
    B_B_im: jax.Array,
    B_C_re: jax.Array,
    B_C_im: jax.Array,
    B_log_dt: jax.Array,
    B_Dskip: jax.Array,
):
    del B_u
    return _run(A_x, A_wqkv, A_w_phi, A_wo, B_A_re, B_A_im, B_B_re, B_B_im,
                B_C_re, B_C_im, B_log_dt, B_Dskip)
```

```python
import functools
import math

import jax
import jax.numpy as jnp
import numpy as np
from jax import lax
import jax.experimental.pallas as pl
import jax.experimental.pallas.tpu as pltpu

S = 2048
D = 512
NS = 128
NA = 16
NK = 16
NFFT = 4096
LOG2E = 1.4426950408889634
F32 = jnp.float32
BF16 = jnp.bfloat16


def _np_constants():
    k1 = np.arange(NK)[:, None] + 0.5
    a = np.arange(NA)[None, :]
    ang = -2.0 * np.pi * k1 * a / 32.0
    f1 = np.concatenate([np.cos(ang), np.sin(ang)], axis=0)
    l1 = np.kron(f1, np.eye(8))
    l1inv = l1.T * (2.0 / NFFT)
    b = np.arange(128)[None, :, None]
    k2 = np.arange(128)[None, None, :]
    kk = (np.arange(NK)[:, None, None] + 0.5) + 32.0 * k2
    ang = -2.0 * np.pi * ((b * kk) % NFFT) / NFFT
    mr, mi = np.cos(ang), np.sin(ang)
    g = np.concatenate([np.concatenate([mr, mi], axis=2),
                        np.concatenate([-mi, mr], axis=2)], axis=1)
    sel = []
    for step in (2, 4, 8):
        m = np.zeros((128, 128), np.float32)
        for j in range(128):
            q, r = divmod(j, step)
            if r * 2 > step or (r * 2 == step and q % 2 == 1):
                q += 1
            src = q * step
            m[src if src < 128 else 1, j] = 1.0
        sel.append(m)
    sel = np.stack(sel, axis=0)
    e = np.zeros((128, 128), np.float32)
    for f in range(16):
        for h in range(8):
            e[f * 8 + h, f] = 1.0
    perm = np.zeros((128, 128), np.float32)
    for d in range(16):
        for h in range(8):
            perm[d * 8 + h, h * 16 + d] = 1.0
    l1inv = l1inv.reshape(128, 2, 128).transpose(1, 0, 2)
    g = np.stack([mr, mi - mr, mr + mi], 1).reshape(NK * 3, 128, 128)
    return (l1.astype(np.float32), l1inv.astype(np.float32), g.astype(np.float32),
            sel.astype(np.float32), e, perm)


_L1, _L1INV, _G, _SEL, _E, _PERM = _np_constants()


def _nt(a, b):
    return lax.dot_general(a, b, (((1,), (1,)), ((), ())), preferred_element_type=F32)


def _nn(a, b):
    return jnp.dot(a, b, preferred_element_type=F32)


def _cmul(ar, ai, br, bi):
    return ar * br - ai * bi, ar * bi + ai * br


def _layernorm_t(x):
    m = jnp.mean(x, axis=0, keepdims=True)
    xc = x - m
    v = jnp.mean(xc * xc, axis=0, keepdims=True)
    return xc * lax.rsqrt(v + 1e-5)


FLAGS = {}
U_KGEN = 4
KSPLIT = (4, 12, 8, 8)
KRING = 4
KLAG = 2
U_S1 = 8
U_LAST = 16
TS = 512
U_MID = 4
RC = 256


def _cat(xs, axis):
    return xs[0] if len(xs) == 1 else jnp.concatenate(xs, axis=axis)


def _kernel(x_hbm, wqkv_hbm, wphi_ref, wo_hbm, are_ref, aim_ref, bre_ref, bim_ref,
            cre_ref, cim_ref, ldt_ref, dsk_ref, l1_ref, l1inv_ref, g_hbm, sel_ref,
            e_ref, perm_ref, o_hbm,
            xt, ut, ub, phiq, phik, vt, s1, s1k, s2, kf, kt, zr, zi, wt, wot, dskb, kvl, kmat,
            x_ref, wqkv_ref, wo_ref, g_ref, o_ref, sems):
    NT = S // TS
    NH = TS // 128
    sub8 = lax.broadcasted_iota(jnp.int32, (8, 128), 0)
    cp_w = pltpu.make_async_copy(wqkv_hbm, wqkv_ref, sems.at[0])
    cp_wo = pltpu.make_async_copy(wo_hbm, wo_ref, sems.at[1])

    def cp_x(i):
        c0 = i * TS if isinstance(i, int) else pl.multiple_of(i * TS, TS)
        return pltpu.make_async_copy(x_hbm.at[pl.ds(c0, TS), :], x_ref.at[pl.ds(c0, TS), :],
                                     sems.at[4 + NT + i])
    cp_g = pltpu.make_async_copy(g_hbm, g_ref, sems.at[3])
    cp_w.start()
    cp_wo.start()

    def dft_fwd(src, k, rows):
        k1 = _nn(src[3 * k + 2, rows, :], g_ref[3 * k])
        k2 = _nn(src[3 * k, rows, :], g_ref[3 * k + 1])
        k3 = _nn(src[3 * k + 1, rows, :], g_ref[3 * k + 2])
        return k1 - k3, k1 + k2

    dskb[...] = jnp.broadcast_to(dsk_ref[...].astype(F32)[None, :], (128, D)).T
    dt = jnp.exp(ldt_ref[...].astype(F32)[None, :]).astype(BF16).astype(F32)
    dt = jnp.broadcast_to(dt, (128, D)).T
    lr = dt * are_ref[...].astype(F32)
    li = dt * aim_ref[...].astype(F32)
    mag = jnp.exp(lr)
    pr, pi = mag * jnp.cos(li), mag * jnp.sin(li)
    for k in range(11):
        zr[k] = pr
        zi[k] = pi
        if k < 10:
            pr, pi = pr * pr - pi * pi, 2.0 * pr * pi
    wr, wi = _cmul(cre_ref[...].astype(F32), cim_ref[...].astype(F32),
                   dt * bre_ref[...].astype(F32), dt * bim_ref[...].astype(F32))
    zr[11] = wr
    zi[11] = -wi

    row_h = lax.broadcasted_iota(jnp.int32, (128, 128), 0) % 8
    col_h16 = lax.broadcasted_iota(jnp.int32, (128, 128), 1) // 16
    col_h8 = lax.broadcasted_iota(jnp.int32, (128, 128), 1) % 8
    cp_w.wait()
    cp_wo.wait()
    for i in range(NT):
        cp_x(i).start()
    wphi = wphi_ref[...].reshape(D, 16)
    for g in range(4):
        m1 = wphi[g * 128:(g + 1) * 128, :]
        pphi = _nt(e_ref[:, 0:16], m1)
        pphi = jnp.where(row_h == col_h16, pphi, 0.0).astype(BF16)
        for j in range(3):
            w = wqkv_ref[:, j * D + g * 128: j * D + (g + 1) * 128]
            r = _nt(pphi, w) * LOG2E if j < 2 else _nt(perm_ref[...], w)
            r = r.astype(BF16)
            for kk in range(4):
                wt[kk, g * 384 + j * 128: g * 384 + (j + 1) * 128, :] = r[:, kk * 128:(kk + 1) * 128]
        wo_p = _nn(perm_ref[...], wo_ref[g * 128:(g + 1) * 128, :])
        wot[g] = wo_p.T.astype(BF16)

    lane16 = lax.broadcasted_iota(jnp.int32, (NA, 128), 1)
    row16 = lax.broadcasted_iota(jnp.int32, (NA, 128), 0)
    keep_lo = (lane16 < 64) & ~((lane16 == 1) & (row16 >= 2))

    def kgen_one(d, slot):
        def bc(k):
            return (jnp.broadcast_to(zr[k, pl.ds(d, 1), :], (8, 128)),
                    jnp.broadcast_to(zi[k, pl.ds(d, 1), :], (8, 128)))

        def selbit(k, bit):
            r, i = bc(k)
            m = (sub8 & bit) != 0
            return jnp.where(m, r, 1.0), jnp.where(m, i, 0.0)

        def cmulc(ar, an, br, bi):
            return ar * br + an * bi, an * br - ar * bi
        yr, yi = selbit(0, 1)
        yr, yi = _cmul(yr, yi, *selbit(1, 2))
        yr, yi = _cmul(yr, yi, *selbit(2, 4))
        ys = [(yr, yi)]
        for k in (3, 4, 5):
            m = bc(k)
            ys = ys + [_cmul(a, b, *m) for a, b in ys]
        z64 = bc(6)
        ys = ys + [z64, z64]
        xr, xn = bc(11)
        xr, xn = cmulc(xr, xn, *selbit(7, 1))
        xr, xn = cmulc(xr, xn, *selbit(8, 2))
        xr, xn = cmulc(xr, xn, *selbit(9, 4))
        xs = [(xr, xn), cmulc(xr, xn, *bc(10))]
        xs = xs + [cmulc(a, b, *z64) for a, b in xs]
        kmat[slot * 2] = _cat([a for a, _ in ys] + [a for a, _ in xs], 0).astype(BF16)
        kmat[slot * 2 + 1] = _cat([b for _, b in ys] + [b for _, b in xs], 0).astype(BF16)

    def kgen_dot(slot):
        ymat = _cat([kmat[slot * 2, 0:80, :], kmat[slot * 2 + 1, 0:80, :]], 1)
        xmat = _cat([kmat[slot * 2, 80:112, :], kmat[slot * 2 + 1, 80:112, :]], 1)
        out = _nt(xmat, ymat)
        out = _cat([out, jnp.zeros((32, 48), F32)], 1)
        hi = pltpu.roll(out[16:32], 64, 1)
        return jnp.where(keep_lo, out[0:16], hi)

    def kgen_build(m, par):
        for j in range(U_KGEN):
            kgen_one(m * U_KGEN + j, par * U_KGEN + j)

    def kgen_dots(m, par):
        res = [kgen_dot(par * U_KGEN + j) for j in range(U_KGEN)]
        for j in range(U_KGEN):
            kt[pl.ds(m * U_KGEN + j, NA, stride=D), :] = res[j]

    class Ticker:
        def __init__(self, base, nstep, npts):
            self.ops = []
            for n in range(nstep):
                m = base + n
                for j in range(U_KGEN):
                    self.ops.append(functools.partial(
                        kgen_dot_store, jnp.maximum(m - KLAG, 0) * U_KGEN + j,
                        ((n - KLAG) % KRING) * U_KGEN + j))
                    self.ops.append(functools.partial(
                        kgen_one, m * U_KGEN + j, (n % KRING) * U_KGEN + j))
            self.npts, self.i, self.done = npts, 0, 0

        def __call__(self):
            self.i += 1
            tgt = len(self.ops) * self.i // self.npts
            for op in self.ops[self.done:tgt]:
                op()
            self.done = tgt

    def kgen_dot_store(d, slot):
        kt[pl.ds(d, NA, stride=D), :] = kgen_dot(slot)

    def no_tick():
        pass

    KP1, KKV, KP2, KS1 = KSPLIT
    assert 4 * (KP1 + KKV + KP2 + KS1) * U_KGEN == D
    kmat[...] = jnp.zeros(kmat.shape, BF16)

    def stage1(load, dst, hook=None):
        def body(i, carry):
            tick = hook(i) if hook is not None else no_tick
            for j in range(U_S1):
                base = (i * U_S1 + j) * 16
                outs = []
                for h in range(2):
                    r0 = pl.multiple_of(base + h * 8, 8)
                    rhs = _cat([load(r0, a) for a in range(NA)], 0).astype(BF16)
                    outs.append(_nn(l1_ref[...], rhs))
                    tick()
                r0 = pl.multiple_of(base, 16)
                for k in range(NK):
                    re = _cat([o[k * 8:k * 8 + 8] for o in outs], 0)
                    im = _cat([o[128 + k * 8:128 + k * 8 + 8] for o in outs], 0)
                    dst[k * 3, pl.ds(r0, 16), :] = re.astype(BF16)
                    dst[k * 3 + 1, pl.ds(r0, 16), :] = im.astype(BF16)
                    dst[k * 3 + 2, pl.ds(r0, 16), :] = (re + im).astype(BF16)
            return carry
        lax.fori_loop(0, D // 16 // U_S1, body, 0)

    def k_finish():
        cp_g.wait()
        for q in range(KLAG, 0, -1):
            kgen_dots(D // U_KGEN - q, (-q) % KRING)
        for a in range(2, NA):
            c = 0 if a < 4 else (1 if a < 8 else 2)
            kt[a * D:(a + 1) * D, :] = _nn(kt[a * D:(a + 1) * D, :].astype(BF16), sel_ref[c])

        stage1(lambda r0, a: kt[pl.ds(a * D + r0, 8), :], s1k)

        def kf_body(i, carry):
            for kk in range(2):
                k = i * 2 + kk
                kf[2 * k], kf[2 * k + 1] = dft_fwd(s1k, k, slice(None))
            return carry
        lax.fori_loop(0, NK // 2, kf_body, 0)

    cp_g.start()

    def xin(i, carry):
        cp_x(i).wait()
        c0 = pl.multiple_of(i * TS, TS)
        xt[:, pl.ds(c0, TS)] = x_ref[pl.ds(c0, TS), :].astype(F32).T
        return carry
    lax.fori_loop(0, NT, xin, 0)

    def softmax_pair(p):
        ps = [p[f * 8:(f + 1) * 8] for f in range(16)]
        mx = functools.reduce(jnp.maximum, ps)
        mn = functools.reduce(jnp.minimum, ps)
        ep = [jnp.exp2(t - mx) for t in ps]
        en = [jnp.exp2(mn - t) for t in ps]
        rp = 1.0 / functools.reduce(jnp.add, ep)
        rn = 1.0 / functools.reduce(jnp.add, en)
        return _cat([t * rp for t in ep] + [t * rn for t in en], 0)

    def ln_to_ub(i, slot):
        c0 = pl.multiple_of(i * TS, TS)
        for h in range(NH):
            u = _layernorm_t(xt[:, pl.ds(c0 + h * 128, 128)]).astype(BF16)
            ub[slot * NH + h] = u

    def layer_a(with_kgen):
        ln_to_ub(0, 0)

        def p1(i, carry):
            slot = i % 2
            tick = Ticker(i * KP1, KP1, 48) if with_kgen else no_tick
            for g in range(4):
                if g == 2:
                    ln_to_ub(jnp.minimum(i + 1, NT - 1), 1 - slot)
                for h in range(NH):
                    n = g * NH + h
                    t = i * NH + h

                    def proj(j):
                        r0 = g * 384 + j * 128
                        w = _cat([wt[kk, r0:r0 + 128, :] for kk in range(4)], 1)
                        return _nn(w, ub[slot * NH + h])

                    pq = proj(0)
                    tick()
                    pk = proj(1)
                    tick()
                    phiq[t, g * 256:(g + 1) * 256, :] = softmax_pair(pq).astype(BF16)
                    pv = proj(2)
                    tick()
                    phik[t, g * 256:(g + 1) * 256, :] = softmax_pair(pk).astype(BF16)
                    vt[t, g * 128:(g + 1) * 128, :] = pv.astype(BF16)
            return carry
        lax.fori_loop(0, NT, p1, 0)

        rowi = lax.broadcasted_iota(jnp.int32, (144, 256), 0)
        coli = lax.broadcasted_iota(jnp.int32, (144, 256), 1)
        kvmask = (rowi % 8 == coli % 8) & (rowi < 136)
        ones = jnp.ones((16, 128), BF16)

        def kv_body(g, carry):
            tick = Ticker(4 * KP1 + g * KKV, KKV, 16) if with_kgen else no_tick
            acc = None
            for c in range(S // 128):
                lhs = _cat([vt[c, pl.ds(pl.multiple_of(g * 128, 128), 128), :], ones], 0)
                r = _nt(lhs, phik[c, pl.ds(pl.multiple_of(g * 256, 256), 256), :])
                acc = r if acc is None else acc + r
                tick()
            t = jnp.where(kvmask, acc, 0.0).astype(BF16)
            kvl[g * 2] = t[:, 0:128]
            kvl[g * 2 + 1] = t[:, 128:256]
            return carry
        lax.fori_loop(0, 4, kv_body, 0)

        NP2 = 4 if with_kgen else 8

        def p2(i, carry):
            tick = Ticker(4 * (KP1 + KKV) + i * KP2, KP2, 5 * NP2) if with_kgen else no_tick

            def num(h):
                os_ = []
                for g in range(4):
                    nd = _nn(_cat([kvl[g * 2], kvl[g * 2 + 1]], 1),
                             phiq[i * NP2 + h, g * 256:(g + 1) * 256, :])
                    r = 1.0 / (nd[128:136] + 1e-6)
                    os_ += [nd[d * 8:(d + 1) * 8] * r for d in range(16)]
                    tick()
                return _cat(os_, 0).astype(BF16)

            def fin(h, o):
                c0 = pl.multiple_of((i * NP2 + h) * 128, 128)
                w = _cat([wot[g] for g in range(4)], 1)
                xn = xt[:, pl.ds(c0, 128)] + _nn(w, o)
                xt[:, pl.ds(c0, 128)] = xn
                ut[:, pl.ds(c0, 128)] = _layernorm_t(xn)
                tick()

            prev = num(0)
            for h in range(1, NP2):
                cur = num(h)
                fin(h - 1, prev)
                prev = cur
            fin(NP2 - 1, prev)
            return carry
        lax.fori_loop(0, S // 128 // NP2, p2, 0)

    def layer_b(first):
        def hook(i):
            return Ticker(4 * (KP1 + KKV + KP2) + i * KS1, KS1, 2 * U_S1)
        stage1(lambda r0, a: ut[pl.ds(r0, 8), a * 128:(a + 1) * 128], s1, hook if first else None)
        if first:
            k_finish()

        def mid(i, carry):
            items = [(i * U_MID + kk, c) for kk in range(U_MID) for c in range(D // RC)]

            def fwd(k, c):
                rows = pl.ds(c * RC, RC)
                zr_, zi_ = dft_fwd(s1, k, rows)
                yr, yi = _cmul(zr_, zi_, kf[2 * k, rows, :], kf[2 * k + 1, rows, :])
                return yr.astype(BF16), yi.astype(BF16), (yr + yi).astype(BF16)

            def inv(k, c, y):
                rows = pl.ds(c * RC, RC)
                j1 = _nt(y[2], g_ref[3 * k])
                s2[2 * k, rows, :] = j1 + _nt(y[1], g_ref[3 * k + 1])
                s2[2 * k + 1, rows, :] = j1 - _nt(y[0], g_ref[3 * k + 2])
            prev = fwd(*items[0])
            for n in range(1, len(items)):
                cur = fwd(*items[n])
                inv(*items[n - 1], prev)
                prev = cur
            inv(*items[-1], prev)
            return carry
        lax.fori_loop(0, NK // U_MID, mid, 0)

        def last(i, carry):
            for j in range(U_LAST):
                r0 = pl.multiple_of((i * U_LAST + j) * 8, 8)
                rhs = _cat([s2[2 * k + ri, pl.ds(r0, 8), :] for ri in range(2) for k in range(NK)],
                           0).astype(BF16)
                y = _nn(_cat([l1inv_ref[0], l1inv_ref[1]], 1), rhs)
                dk = dskb[pl.ds(r0, 8), :]
                for a in range(NA):
                    sl = (pl.ds(r0, 8), slice(a * 128, (a + 1) * 128))
                    xt[sl] = xt[sl] + (y[a * 8:(a + 1) * 8] + ut[sl] * dk)
            return carry
        lax.fori_loop(0, D // 8 // U_LAST, last, 0)

    layer_a(True)
    layer_b(True)
    layer_a(False)
    layer_b(False)

    def xout(i, carry):
        c0 = pl.multiple_of(i * TS, TS)
        o_ref[pl.ds(c0, TS), :] = xt[:, pl.ds(c0, TS)].T.astype(BF16)
        pltpu.make_async_copy(o_ref.at[pl.ds(c0, TS), :], o_hbm.at[pl.ds(c0, TS), :],
                              sems.at[4 + i]).start()
        return carry
    lax.fori_loop(0, NT, xout, 0)
    for i in range(NT):
        pltpu.make_async_copy(o_ref.at[pl.ds(i * TS, TS), :], o_hbm.at[pl.ds(i * TS, TS), :],
                              sems.at[4 + i]).wait()


def _run(A_x, A_wqkv, A_w_phi, A_wo, B_A_re, B_A_im, B_B_re, B_B_im, B_C_re, B_C_im,
         B_log_dt, B_Dskip, interpret=False):
    consts = [jnp.asarray(c, dtype=BF16) for c in (_L1, _L1INV, _G, _SEL, _E, _PERM)]
    scratch = [
        pltpu.VMEM((D, S), F32),
        pltpu.VMEM((D, S), F32),
        pltpu.VMEM((2 * TS // 128, D, 128), BF16),
        pltpu.VMEM((S // 128, 2 * D, 128), BF16),
        pltpu.VMEM((S // 128, 2 * D, 128), BF16),
        pltpu.VMEM((S // 128, D, 128), BF16),
        pltpu.VMEM((NK * 3, D, 128), BF16),
        pltpu.VMEM((NK * 3, D, 128), BF16),
        pltpu.VMEM((NK * 2, D, 128), F32),
        pltpu.VMEM((NK * 2, D, 128), F32),
        pltpu.VMEM((NA * D, 128), F32),
        pltpu.VMEM((12, D, NS), F32),
        pltpu.VMEM((12, D, NS), F32),
        pltpu.VMEM((4, 3 * D, 128), BF16),
        pltpu.VMEM((4, D, 128), BF16),
        pltpu.VMEM((D, 128), F32),
        pltpu.VMEM((8, 144, 128), BF16),
        pltpu.VMEM((2 * KRING * U_KGEN, 112, 128), BF16),
        pltpu.VMEM((S, D), BF16),
        pltpu.VMEM((D, 3 * D), BF16),
        pltpu.VMEM((D, D), BF16),
        pltpu.VMEM((NK * 3, 128, 128), BF16),
        pltpu.VMEM((S, D), BF16),
        pltpu.SemaphoreType.DMA((4 + 2 * (S // TS),)),
    ]
    out = pl.pallas_call(
        _kernel,
        out_shape=jax.ShapeDtypeStruct((S, D), BF16),
        in_specs=[pl.BlockSpec(memory_space=pl.ANY) if i in (0, 1, 3, 14)
                  else pl.BlockSpec(memory_space=pltpu.VMEM) for i in range(18)],
        out_specs=pl.BlockSpec(memory_space=pl.ANY),
        scratch_shapes=scratch,
        compiler_params=pltpu.CompilerParams(vmem_limit_bytes=110 * 2**20, flags=FLAGS),
        interpret=interpret,
        name="hedgehog_s4",
    )(A_x.reshape(S, D), A_wqkv, A_w_phi, A_wo, B_A_re, B_A_im, B_B_re,
      B_B_im, B_C_re, B_C_im, B_log_dt, B_Dskip, *consts)
    return out.reshape(1, S, D)


@jax.jit
def pallas_interleave_layers__linear_kernel_hedgehog__ssm_conv_s4__prompt_kernel(
    A_x: jax.Array,
    A_wqkv: jax.Array,
    A_w_phi: jax.Array,
    A_wo: jax.Array,
    B_u: jax.Array,
    B_A_re: jax.Array,
    B_A_im: jax.Array,
    B_B_re: jax.Array,
    B_B_im: jax.Array,
    B_C_re: jax.Array,
    B_C_im: jax.Array,
    B_log_dt: jax.Array,
    B_Dskip: jax.Array,
):
    del B_u
    return _run(A_x, A_wqkv, A_w_phi, A_wo, B_A_re, B_A_im, B_B_re, B_B_im,
                B_C_re, B_C_im, B_log_dt, B_Dskip)
```

```python
import functools

import jax
import jax.numpy as jnp
import numpy as np
from jax import lax
import jax.experimental.pallas as pl
import jax.experimental.pallas.tpu as pltpu

S = 2048
D = 512
NS = 128
NA = 16
NK = 16
NFFT = 4096
LOG2E = 1.4426950408889634
F32 = jnp.float32
BF16 = jnp.bfloat16


def _np_constants():
    k1 = np.arange(NK)[:, None] + 0.5
    a = np.arange(NA)[None, :]
    ang = -2.0 * np.pi * k1 * a / 32.0
    f1 = np.concatenate([np.cos(ang), np.sin(ang)], axis=0)
    l1 = np.kron(f1, np.eye(8))
    l1inv = l1.T * (2.0 / NFFT)
    b = np.arange(128)[None, :, None]
    k2 = np.arange(128)[None, None, :]
    kk = (np.arange(NK)[:, None, None] + 0.5) + 32.0 * k2
    ang = -2.0 * np.pi * ((b * kk) % NFFT) / NFFT
    mr, mi = np.cos(ang), np.sin(ang)
    g = np.concatenate([np.concatenate([mr, mi], axis=2),
                        np.concatenate([-mi, mr], axis=2)], axis=1)
    sel = []
    for step in (2, 4, 8):
        m = np.zeros((128, 128), np.float32)
        for j in range(128):
            q, r = divmod(j, step)
            if r * 2 > step or (r * 2 == step and q % 2 == 1):
                q += 1
            src = q * step
            m[src if src < 128 else 1, j] = 1.0
        sel.append(m)
    sel = np.stack(sel, axis=0)
    e = np.zeros((128, 128), np.float32)
    for f in range(16):
        for h in range(8):
            e[f * 8 + h, f] = 1.0
    perm = np.zeros((128, 128), np.float32)
    for d in range(16):
        for h in range(8):
            perm[d * 8 + h, h * 16 + d] = 1.0
    l1inv = l1inv.reshape(128, 2, 128).transpose(1, 0, 2)
    g = np.stack([mr, mi - mr, mr + mi], 1).reshape(NK * 3, 128, 128)
    return (l1.astype(np.float32), l1inv.astype(np.float32), g.astype(np.float32),
            sel.astype(np.float32), e, perm)


_L1, _L1INV, _G, _SEL, _E, _PERM = _np_constants()


def _nt(a, b):
    return lax.dot_general(a, b, (((1,), (1,)), ((), ())), preferred_element_type=F32)


def _nn(a, b):
    return jnp.dot(a, b, preferred_element_type=F32)


def _cmul(ar, ai, br, bi):
    return ar * br - ai * bi, ar * bi + ai * br


def _layernorm_t(x):
    m = jnp.mean(x, axis=0, keepdims=True)
    xc = x - m
    v = jnp.mean(xc * xc, axis=0, keepdims=True)
    return xc * lax.rsqrt(v + 1e-5)


FLAGS = {}
U_KGEN = 4
KSPLIT = (0, 12, 8, 12)
U_S1 = 8
U_LAST = 16
TS = 512
U_MID = 4
RC = 256


def _cat(xs, axis):
    return xs[0] if len(xs) == 1 else jnp.concatenate(xs, axis=axis)


def _kernel(x_hbm, wqkv_hbm, wphi_ref, wo_hbm, are_ref, aim_ref, bre_ref, bim_ref,
            cre_ref, cim_ref, ldt_ref, dsk_ref, l1_ref, l1inv_ref, g_hbm, sel_ref,
            e_ref, perm_ref, o_hbm,
            xt, ut, ub, phiq, phik, vt, s1, s1k, s2, kf, kt, zr, zi, wt, wot, dskb, kvl,
            x_ref, wqkv_ref, wo_ref, g_ref, o_ref, sems):
    NT = S // TS
    NH = TS // 128
    sub8 = lax.broadcasted_iota(jnp.int32, (8, 128), 0)
    cp_w = pltpu.make_async_copy(wqkv_hbm, wqkv_ref, sems.at[0])
    cp_wo = pltpu.make_async_copy(wo_hbm, wo_ref, sems.at[1])

    def cp_x(i):
        c0 = i * TS if isinstance(i, int) else pl.multiple_of(i * TS, TS)
        return pltpu.make_async_copy(x_hbm.at[pl.ds(c0, TS), :], x_ref.at[pl.ds(c0, TS), :],
                                     sems.at[4 + NT + i])
    cp_g = pltpu.make_async_copy(g_hbm, g_ref, sems.at[3])
    cp_w.start()
    cp_wo.start()

    def dft_fwd(src, k, rows):
        k1 = _nn(src[3 * k + 2, rows, :], g_ref[3 * k])
        k2 = _nn(src[3 * k, rows, :], g_ref[3 * k + 1])
        k3 = _nn(src[3 * k + 1, rows, :], g_ref[3 * k + 2])
        return k1 - k3, k1 + k2

    dskb[...] = jnp.broadcast_to(dsk_ref[...].astype(F32)[None, :], (128, D)).T
    dt = jnp.exp(ldt_ref[...].astype(F32)[None, :]).astype(BF16).astype(F32)
    dt = jnp.broadcast_to(dt, (128, D)).T
    lr = dt * are_ref[...].astype(F32)
    li = dt * aim_ref[...].astype(F32)
    mag = jnp.exp(lr)
    pr, pi = mag * jnp.cos(li), mag * jnp.sin(li)
    for k in range(11):
        zr[k] = pr
        zi[k] = pi
        if k < 10:
            pr, pi = pr * pr - pi * pi, 2.0 * pr * pi
    wr, wi = _cmul(cre_ref[...].astype(F32), cim_ref[...].astype(F32),
                   dt * bre_ref[...].astype(F32), dt * bim_ref[...].astype(F32))
    zr[11] = wr
    zi[11] = -wi

    row_h = lax.broadcasted_iota(jnp.int32, (128, 128), 0) % 8
    col_h16 = lax.broadcasted_iota(jnp.int32, (128, 128), 1) // 16
    col_h8 = lax.broadcasted_iota(jnp.int32, (128, 128), 1) % 8
    cp_w.wait()
    cp_wo.wait()
    for i in range(NT):
        cp_x(i).start()
    wphi = wphi_ref[...].reshape(D, 16)
    for g in range(4):
        m1 = wphi[g * 128:(g + 1) * 128, :]
        pphi = _nt(e_ref[:, 0:16], m1)
        pphi = jnp.where(row_h == col_h16, pphi, 0.0).astype(BF16)
        for j in range(3):
            w = wqkv_ref[:, j * D + g * 128: j * D + (g + 1) * 128]
            r = _nt(pphi, w) * LOG2E if j < 2 else _nt(perm_ref[...], w)
            r = r.astype(BF16)
            for kk in range(4):
                wt[kk, g * 384 + j * 128: g * 384 + (j + 1) * 128, :] = r[:, kk * 128:(kk + 1) * 128]
        wo_p = _nn(perm_ref[...], wo_ref[g * 128:(g + 1) * 128, :])
        wot[g] = wo_p.T.astype(BF16)

    lane16 = lax.broadcasted_iota(jnp.int32, (NA, 128), 1)
    row16 = lax.broadcasted_iota(jnp.int32, (NA, 128), 0)
    keep_lo = (lane16 < 64) & ~((lane16 == 1) & (row16 >= 2))

    def kgen_one(d):
        def bc(k):
            return (jnp.broadcast_to(zr[k, pl.ds(d, 1), :], (8, 128)),
                    jnp.broadcast_to(zi[k, pl.ds(d, 1), :], (8, 128)))

        def selbit(k, bit):
            r, i = bc(k)
            m = (sub8 & bit) != 0
            return jnp.where(m, r, 1.0), jnp.where(m, i, 0.0)

        def cmulc(ar, an, br, bi):
            return ar * br + an * bi, an * br - ar * bi
        yr, yi = selbit(0, 1)
        yr, yi = _cmul(yr, yi, *selbit(1, 2))
        yr, yi = _cmul(yr, yi, *selbit(2, 4))
        ys = [(yr, yi)]
        for k in (3, 4, 5):
            m = bc(k)
            ys = ys + [_cmul(a, b, *m) for a, b in ys]
        z64 = bc(6)
        ys = ys + [z64, z64]
        xr, xn = bc(11)
        xr, xn = cmulc(xr, xn, *selbit(7, 1))
        xr, xn = cmulc(xr, xn, *selbit(8, 2))
        xr, xn = cmulc(xr, xn, *selbit(9, 4))
        xs = [(xr, xn), cmulc(xr, xn, *bc(10))]
        xs = xs + [cmulc(a, b, *z64) for a, b in xs]
        ymat = _cat([_cat([a for a, _ in ys], 0), _cat([b for _, b in ys], 0)], 1).astype(BF16)
        xmat = _cat([_cat([a for a, _ in xs], 0), _cat([b for _, b in xs], 0)], 1).astype(BF16)
        out = _cat([_nt(xmat, ymat), jnp.zeros((32, 48), F32)], 1)
        res = jnp.where(keep_lo, out[0:16], pltpu.roll(out[16:32], 64, 1))
        kt[pl.ds(d, NA, stride=D), :] = res

    class Ticker:
        def __init__(self, base, nstep, npts):
            self.ops = []
            for n in range(nstep):
                m = base + n
                for j in range(U_KGEN):
                    self.ops.append(functools.partial(kgen_one, m * U_KGEN + j))
            self.npts, self.i, self.done = npts, 0, 0

        def __call__(self):
            self.i += 1
            tgt = len(self.ops) * self.i // self.npts
            for op in self.ops[self.done:tgt]:
                op()
            self.done = tgt

    def no_tick():
        pass

    KP1, KKV, KP2, KS1 = KSPLIT
    assert 4 * (KP1 + KKV + KP2 + KS1) * U_KGEN == D

    def stage1(load, dst, hook=None):
        def body(i, carry):
            tick = hook(i) if hook is not None else no_tick
            for j in range(U_S1):
                base = (i * U_S1 + j) * 16
                outs = []
                for h in range(2):
                    r0 = pl.multiple_of(base + h * 8, 8)
                    rhs = _cat([load(r0, a) for a in range(NA)], 0).astype(BF16)
                    outs.append(_nn(l1_ref[...], rhs))
                    tick()
                r0 = pl.multiple_of(base, 16)
                for k in range(NK):
                    re = _cat([o[k * 8:k * 8 + 8] for o in outs], 0)
                    im = _cat([o[128 + k * 8:128 + k * 8 + 8] for o in outs], 0)
                    dst[k * 3, pl.ds(r0, 16), :] = re.astype(BF16)
                    dst[k * 3 + 1, pl.ds(r0, 16), :] = im.astype(BF16)
                    dst[k * 3 + 2, pl.ds(r0, 16), :] = (re + im).astype(BF16)
            return carry
        lax.fori_loop(0, D // 16 // U_S1, body, 0)

    def k_finish():
        cp_g.wait()
        for a in range(2, NA):
            c = 0 if a < 4 else (1 if a < 8 else 2)
            kt[a * D:(a + 1) * D, :] = _nn(kt[a * D:(a + 1) * D, :].astype(BF16), sel_ref[c])

        stage1(lambda r0, a: kt[pl.ds(a * D + r0, 8), :], s1k)

        def kf_body(i, carry):
            for kk in range(2):
                k = i * 2 + kk
                kf[2 * k], kf[2 * k + 1] = dft_fwd(s1k, k, slice(None))
            return carry
        lax.fori_loop(0, NK // 2, kf_body, 0)

    cp_g.start()

    def xin(i, carry):
        cp_x(i).wait()
        c0 = pl.multiple_of(i * TS, TS)
        xt[:, pl.ds(c0, TS)] = x_ref[pl.ds(c0, TS), :].astype(F32).T
        return carry
    lax.fori_loop(0, NT, xin, 0)

    def softmax_pair(p):
        ps = [p[f * 8:(f + 1) * 8] for f in range(16)]
        mx = functools.reduce(jnp.maximum, ps)
        mn = functools.reduce(jnp.minimum, ps)
        ep = [jnp.exp2(t - mx) for t in ps]
        en = [jnp.exp2(mn - t) for t in ps]
        rp = 1.0 / functools.reduce(jnp.add, ep)
        rn = 1.0 / functools.reduce(jnp.add, en)
        return _cat([t * rp for t in ep] + [t * rn for t in en], 0)

    def ln_to_ub(i, slot):
        c0 = pl.multiple_of(i * TS, TS)
        for h in range(NH):
            u = _layernorm_t(xt[:, pl.ds(c0 + h * 128, 128)]).astype(BF16)
            ub[slot * NH + h] = u

    def layer_a(with_kgen):
        ln_to_ub(0, 0)

        def p1(i, carry):
            slot = i % 2
            tick = Ticker(i * KP1, KP1, 48) if with_kgen else no_tick
            for g in range(4):
                if g == 2:
                    ln_to_ub(jnp.minimum(i + 1, NT - 1), 1 - slot)
                for h in range(NH):
                    n = g * NH + h
                    t = i * NH + h

                    def proj(j):
                        r0 = g * 384 + j * 128
                        w = _cat([wt[kk, r0:r0 + 128, :] for kk in range(4)], 1)
                        return _nn(w, ub[slot * NH + h])

                    pq = proj(0)
                    tick()
                    pk = proj(1)
                    tick()
                    phiq[t, g * 256:(g + 1) * 256, :] = softmax_pair(pq).astype(BF16)
                    pv = proj(2)
                    tick()
                    phik[t, g * 256:(g + 1) * 256, :] = softmax_pair(pk).astype(BF16)
                    vt[t, g * 128:(g + 1) * 128, :] = pv.astype(BF16)
            return carry
        lax.fori_loop(0, NT, p1, 0)

        rowi = lax.broadcasted_iota(jnp.int32, (144, 256), 0)
        coli = lax.broadcasted_iota(jnp.int32, (144, 256), 1)
        kvmask = (rowi % 8 == coli % 8) & (rowi < 136)
        ones = jnp.ones((16, 128), BF16)

        def kv_body(g, carry):
            tick = Ticker(4 * KP1 + g * KKV, KKV, 16) if with_kgen else no_tick
            acc = None
            for c in range(S // 128):
                lhs = _cat([vt[c, pl.ds(pl.multiple_of(g * 128, 128), 128), :], ones], 0)
                r = _nt(lhs, phik[c, pl.ds(pl.multiple_of(g * 256, 256), 256), :])
                acc = r if acc is None else acc + r
                tick()
            t = jnp.where(kvmask, acc, 0.0).astype(BF16)
            kvl[g * 2] = t[:, 0:128]
            kvl[g * 2 + 1] = t[:, 128:256]
            return carry
        lax.fori_loop(0, 4, kv_body, 0)

        NP2 = 4 if with_kgen else 8

        def p2(i, carry):
            tick = Ticker(4 * (KP1 + KKV) + i * KP2, KP2, 5 * NP2) if with_kgen else no_tick

            def num(h):
                os_ = []
                for g in range(4):
                    nd = _nn(_cat([kvl[g * 2], kvl[g * 2 + 1]], 1),
                             phiq[i * NP2 + h, g * 256:(g + 1) * 256, :])
                    r = 1.0 / (nd[128:136] + 1e-6)
                    os_ += [nd[d * 8:(d + 1) * 8] * r for d in range(16)]
                    tick()
                return _cat(os_, 0).astype(BF16)

            def fin(h, o):
                c0 = pl.multiple_of((i * NP2 + h) * 128, 128)
                w = _cat([wot[g] for g in range(4)], 1)
                xn = xt[:, pl.ds(c0, 128)] + _nn(w, o)
                xt[:, pl.ds(c0, 128)] = xn
                ut[:, pl.ds(c0, 128)] = _layernorm_t(xn)
                tick()

            prev = num(0)
            for h in range(1, NP2):
                cur = num(h)
                fin(h - 1, prev)
                prev = cur
            fin(NP2 - 1, prev)
            return carry
        lax.fori_loop(0, S // 128 // NP2, p2, 0)

    def layer_b(first):
        def hook(i):
            return Ticker(4 * (KP1 + KKV + KP2) + i * KS1, KS1, 2 * U_S1)
        stage1(lambda r0, a: ut[pl.ds(r0, 8), a * 128:(a + 1) * 128], s1, hook if first else None)
        if first:
            k_finish()

        def mid(i, carry):
            items = [(i * U_MID + kk, c) for kk in range(U_MID) for c in range(D // RC)]

            def fwd(k, c):
                rows = pl.ds(c * RC, RC)
                zr_, zi_ = dft_fwd(s1, k, rows)
                yr, yi = _cmul(zr_, zi_, kf[2 * k, rows, :], kf[2 * k + 1, rows, :])
                return yr.astype(BF16), yi.astype(BF16), (yr + yi).astype(BF16)

            def inv(k, c, y):
                rows = pl.ds(c * RC, RC)
                j1 = _nt(y[2], g_ref[3 * k])
                s2[2 * k, rows, :] = j1 + _nt(y[1], g_ref[3 * k + 1])
                s2[2 * k + 1, rows, :] = j1 - _nt(y[0], g_ref[3 * k + 2])
            prev = fwd(*items[0])
            for n in range(1, len(items)):
                cur = fwd(*items[n])
                inv(*items[n - 1], prev)
                prev = cur
            inv(*items[-1], prev)
            return carry
        lax.fori_loop(0, NK // U_MID, mid, 0)

        def last(i, carry):
            for j in range(U_LAST):
                r0 = pl.multiple_of((i * U_LAST + j) * 8, 8)
                rhs = _cat([s2[2 * k + ri, pl.ds(r0, 8), :] for ri in range(2) for k in range(NK)],
                           0).astype(BF16)
                y = _nn(_cat([l1inv_ref[0], l1inv_ref[1]], 1), rhs)
                dk = dskb[pl.ds(r0, 8), :]
                for a in range(NA):
                    sl = (pl.ds(r0, 8), slice(a * 128, (a + 1) * 128))
                    xt[sl] = xt[sl] + (y[a * 8:(a + 1) * 8] + ut[sl] * dk)
            return carry
        lax.fori_loop(0, D // 8 // U_LAST, last, 0)

    layer_a(True)
    layer_b(True)
    layer_a(False)
    layer_b(False)

    def xout(i, carry):
        c0 = pl.multiple_of(i * TS, TS)
        o_ref[pl.ds(c0, TS), :] = xt[:, pl.ds(c0, TS)].T.astype(BF16)
        pltpu.make_async_copy(o_ref.at[pl.ds(c0, TS), :], o_hbm.at[pl.ds(c0, TS), :],
                              sems.at[4 + i]).start()
        return carry
    lax.fori_loop(0, NT, xout, 0)
    for i in range(NT):
        pltpu.make_async_copy(o_ref.at[pl.ds(i * TS, TS), :], o_hbm.at[pl.ds(i * TS, TS), :],
                              sems.at[4 + i]).wait()


def _run(A_x, A_wqkv, A_w_phi, A_wo, B_A_re, B_A_im, B_B_re, B_B_im, B_C_re, B_C_im,
         B_log_dt, B_Dskip, interpret=False):
    consts = [jnp.asarray(c, dtype=BF16) for c in (_L1, _L1INV, _G, _SEL, _E, _PERM)]
    scratch = [
        pltpu.VMEM((D, S), F32),
        pltpu.VMEM((D, S), F32),
        pltpu.VMEM((2 * TS // 128, D, 128), BF16),
        pltpu.VMEM((S // 128, 2 * D, 128), BF16),
        pltpu.VMEM((S // 128, 2 * D, 128), BF16),
        pltpu.VMEM((S // 128, D, 128), BF16),
        pltpu.VMEM((NK * 3, D, 128), BF16),
        pltpu.VMEM((NK * 3, D, 128), BF16),
        pltpu.VMEM((NK * 2, D, 128), F32),
        pltpu.VMEM((NK * 2, D, 128), F32),
        pltpu.VMEM((NA * D, 128), F32),
        pltpu.VMEM((12, D, NS), F32),
        pltpu.VMEM((12, D, NS), F32),
        pltpu.VMEM((4, 3 * D, 128), BF16),
        pltpu.VMEM((4, D, 128), BF16),
        pltpu.VMEM((D, 128), F32),
        pltpu.VMEM((8, 144, 128), BF16),
        pltpu.VMEM((S, D), BF16),
        pltpu.VMEM((D, 3 * D), BF16),
        pltpu.VMEM((D, D), BF16),
        pltpu.VMEM((NK * 3, 128, 128), BF16),
        pltpu.VMEM((S, D), BF16),
        pltpu.SemaphoreType.DMA((4 + 2 * (S // TS),)),
    ]
    out = pl.pallas_call(
        _kernel,
        out_shape=jax.ShapeDtypeStruct((S, D), BF16),
        in_specs=[pl.BlockSpec(memory_space=pl.ANY) if i in (0, 1, 3, 14)
                  else pl.BlockSpec(memory_space=pltpu.VMEM) for i in range(18)],
        out_specs=pl.BlockSpec(memory_space=pl.ANY),
        scratch_shapes=scratch,
        compiler_params=pltpu.CompilerParams(vmem_limit_bytes=110 * 2**20, flags=FLAGS),
        interpret=interpret,
        name="hedgehog_s4",
    )(A_x.reshape(S, D), A_wqkv, A_w_phi, A_wo, B_A_re, B_A_im, B_B_re,
      B_B_im, B_C_re, B_C_im, B_log_dt, B_Dskip, *consts)
    return out.reshape(1, S, D)


@jax.jit
def pallas_interleave_layers__linear_kernel_hedgehog__ssm_conv_s4__prompt_kernel(
    A_x: jax.Array,
    A_wqkv: jax.Array,
    A_w_phi: jax.Array,
    A_wo: jax.Array,
    B_u: jax.Array,
    B_A_re: jax.Array,
    B_A_im: jax.Array,
    B_B_re: jax.Array,
    B_B_im: jax.Array,
    B_C_re: jax.Array,
    B_C_im: jax.Array,
    B_log_dt: jax.Array,
    B_Dskip: jax.Array,
):
    del B_u
    return _run(A_x, A_wqkv, A_w_phi, A_wo, B_A_re, B_A_im, B_B_re, B_B_im,
                B_C_re, B_C_im, B_log_dt, B_Dskip)
```

```python
import functools

import jax
import jax.numpy as jnp
import numpy as np
from jax import lax
import jax.experimental.pallas as pl
import jax.experimental.pallas.tpu as pltpu

S = 2048
D = 512
NS = 128
NA = 16
NK = 16
NFFT = 4096
LOG2E = 1.4426950408889634
F32 = jnp.float32
BF16 = jnp.bfloat16


def _np_constants():
    k1 = np.arange(NK)[:, None] + 0.5
    a = np.arange(NA)[None, :]
    ang = -2.0 * np.pi * k1 * a / 32.0
    f1 = np.concatenate([np.cos(ang), np.sin(ang)], axis=0)
    l1 = np.kron(f1, np.eye(8))
    l1inv = l1.T * (2.0 / NFFT)
    b = np.arange(128)[None, :, None]
    k2 = np.arange(128)[None, None, :]
    kk = (np.arange(NK)[:, None, None] + 0.5) + 32.0 * k2
    ang = -2.0 * np.pi * ((b * kk) % NFFT) / NFFT
    mr, mi = np.cos(ang), np.sin(ang)
    g = np.concatenate([np.concatenate([mr, mi], axis=2),
                        np.concatenate([-mi, mr], axis=2)], axis=1)
    sel = []
    for step in (2, 4, 8):
        m = np.zeros((128, 128), np.float32)
        for j in range(128):
            q, r = divmod(j, step)
            if r * 2 > step or (r * 2 == step and q % 2 == 1):
                q += 1
            src = q * step
            m[src if src < 128 else 1, j] = 1.0
        sel.append(m)
    sel = np.stack(sel, axis=0)
    e = np.zeros((128, 128), np.float32)
    for f in range(16):
        for h in range(8):
            e[f * 8 + h, f] = 1.0
    perm = np.zeros((128, 128), np.float32)
    for d in range(16):
        for h in range(8):
            perm[d * 8 + h, h * 16 + d] = 1.0
    l1inv = l1inv.reshape(128, 2, 128).transpose(1, 0, 2)
    g = np.stack([mr, mi - mr, mr + mi], 1).reshape(NK * 3, 128, 128)
    return (l1.astype(np.float32), l1inv.astype(np.float32), g.astype(np.float32),
            sel.astype(np.float32), e, perm)


_L1, _L1INV, _G, _SEL, _E, _PERM = _np_constants()


def _nt(a, b):
    return lax.dot_general(a, b, (((1,), (1,)), ((), ())), preferred_element_type=F32)


def _nn(a, b):
    return jnp.dot(a, b, preferred_element_type=F32)


def _cmul(ar, ai, br, bi):
    return ar * br - ai * bi, ar * bi + ai * br


def _layernorm_t(x):
    m = jnp.mean(x, axis=0, keepdims=True)
    xc = x - m
    v = jnp.mean(xc * xc, axis=0, keepdims=True)
    return xc * lax.rsqrt(v + 1e-5)


FLAGS = {}
U_KGEN = 4
KSPLIT = (0, 12, 8, 24)
U_S1 = 16
U_LAST = 32
TS = 512
U_MID = 8
RC = 256


def _cat(xs, axis):
    return xs[0] if len(xs) == 1 else jnp.concatenate(xs, axis=axis)


def _kernel(x_hbm, wqkv_hbm, wphi_ref, wo_hbm, are_ref, aim_ref, bre_ref, bim_ref,
            cre_ref, cim_ref, ldt_ref, dsk_ref, l1_ref, l1inv_ref, g_hbm, sel_ref,
            e_ref, perm_ref, o_hbm,
            xt, ut, ub, phiq, phik, vt, s1, s1k, s2, kf, kt, zr, zi, wt, wot, dskb, kvl,
            x_ref, wqkv_ref, wo_ref, g_ref, o_ref, sems):
    NT = S // TS
    NH = TS // 128
    sub8 = lax.broadcasted_iota(jnp.int32, (8, 128), 0)
    cp_w = pltpu.make_async_copy(wqkv_hbm, wqkv_ref, sems.at[0])
    cp_wo = pltpu.make_async_copy(wo_hbm, wo_ref, sems.at[1])

    def cp_x(i):
        c0 = i * TS if isinstance(i, int) else pl.multiple_of(i * TS, TS)
        return pltpu.make_async_copy(x_hbm.at[pl.ds(c0, TS), :], x_ref.at[pl.ds(c0, TS), :],
                                     sems.at[4 + NT + i])
    cp_g = pltpu.make_async_copy(g_hbm, g_ref, sems.at[3])
    cp_w.start()
    cp_wo.start()

    def dft_fwd(src, k, rows):
        k1 = _nn(src[3 * k + 2, rows, :], g_ref[3 * k])
        k2 = _nn(src[3 * k, rows, :], g_ref[3 * k + 1])
        k3 = _nn(src[3 * k + 1, rows, :], g_ref[3 * k + 2])
        return k1 - k3, k1 + k2

    dskb[...] = jnp.broadcast_to(dsk_ref[...].astype(F32)[None, :], (128, D)).T
    dt = jnp.exp(ldt_ref[...].astype(F32)[None, :]).astype(BF16).astype(F32)
    dt = jnp.broadcast_to(dt, (128, D)).T
    lr = dt * are_ref[...].astype(F32)
    li = dt * aim_ref[...].astype(F32)
    mag = jnp.exp(lr)
    pr, pi = mag * jnp.cos(li), mag * jnp.sin(li)
    for k in range(11):
        zr[k] = pr
        zi[k] = pi
        if k < 10:
            pr, pi = pr * pr - pi * pi, 2.0 * pr * pi
    wr, wi = _cmul(cre_ref[...].astype(F32), cim_ref[...].astype(F32),
                   dt * bre_ref[...].astype(F32), dt * bim_ref[...].astype(F32))
    zr[11] = wr
    zi[11] = -wi

    row_h = lax.broadcasted_iota(jnp.int32, (128, 128), 0) % 8
    col_h16 = lax.broadcasted_iota(jnp.int32, (128, 128), 1) // 16
    col_h8 = lax.broadcasted_iota(jnp.int32, (128, 128), 1) % 8
    cp_w.wait()
    cp_wo.wait()
    for i in range(NT):
        cp_x(i).start()
    wphi = wphi_ref[...].reshape(D, 16)
    for g in range(4):
        m1 = wphi[g * 128:(g + 1) * 128, :]
        pphi = _nt(e_ref[:, 0:16], m1)
        pphi = jnp.where(row_h == col_h16, pphi, 0.0).astype(BF16)
        for j in range(3):
            w = wqkv_ref[:, j * D + g * 128: j * D + (g + 1) * 128]
            r = _nt(pphi, w) * LOG2E if j < 2 else _nt(perm_ref[...], w)
            r = r.astype(BF16)
            for kk in range(4):
                wt[kk, g * 384 + j * 128: g * 384 + (j + 1) * 128, :] = r[:, kk * 128:(kk + 1) * 128]
        wo_p = _nn(perm_ref[...], wo_ref[g * 128:(g + 1) * 128, :])
        wot[g] = wo_p.T.astype(BF16)

    lane16 = lax.broadcasted_iota(jnp.int32, (NA, 128), 1)
    row16 = lax.broadcasted_iota(jnp.int32, (NA, 128), 0)
    keep_lo = (lane16 < 64) & ~((lane16 == 1) & (row16 >= 2))

    def kgen_one(d):
        def bc(k):
            return (jnp.broadcast_to(zr[k, pl.ds(d, 1), :], (8, 128)),
                    jnp.broadcast_to(zi[k, pl.ds(d, 1), :], (8, 128)))

        def selbit(k, bit):
            r, i = bc(k)
            m = (sub8 & bit) != 0
            return jnp.where(m, r, 1.0), jnp.where(m, i, 0.0)

        def cmulc(ar, an, br, bi):
            return ar * br + an * bi, an * br - ar * bi
        yr, yi = selbit(0, 1)
        yr, yi = _cmul(yr, yi, *selbit(1, 2))
        yr, yi = _cmul(yr, yi, *selbit(2, 4))
        ys = [(yr, yi)]
        for k in (3, 4, 5):
            m = bc(k)
            ys = ys + [_cmul(a, b, *m) for a, b in ys]
        z64 = bc(6)
        ys = ys + [z64, z64]
        xr, xn = bc(11)
        xr, xn = cmulc(xr, xn, *selbit(7, 1))
        xr, xn = cmulc(xr, xn, *selbit(8, 2))
        xr, xn = cmulc(xr, xn, *selbit(9, 4))
        xs = [(xr, xn), cmulc(xr, xn, *bc(10))]
        xs = xs + [cmulc(a, b, *z64) for a, b in xs]
        ymat = _cat([_cat([a for a, _ in ys], 0), _cat([b for _, b in ys], 0)], 1).astype(BF16)
        xmat = _cat([_cat([a for a, _ in xs], 0), _cat([b for _, b in xs], 0)], 1).astype(BF16)
        out = _cat([_nt(xmat, ymat), jnp.zeros((32, 48), F32)], 1)
        res = jnp.where(keep_lo, out[0:16], pltpu.roll(out[16:32], 64, 1))
        kt[pl.ds(d, NA, stride=D), :] = res

    class Ticker:
        def __init__(self, base, nstep, npts):
            self.ops = []
            for n in range(nstep):
                m = base + n
                for j in range(U_KGEN):
                    self.ops.append(functools.partial(kgen_one, m * U_KGEN + j))
            self.npts, self.i, self.done = npts, 0, 0

        def __call__(self):
            self.i += 1
            tgt = len(self.ops) * self.i // self.npts
            for op in self.ops[self.done:tgt]:
                op()
            self.done = tgt

    def no_tick():
        pass

    KP1, KKV, KP2, KS1 = KSPLIT
    assert 4 * (KP1 + KKV + KP2) * U_KGEN + 2 * KS1 * U_KGEN == D

    def stage1(load, dst, hook=None):
        def body(i, carry):
            tick = hook(i) if hook is not None else no_tick
            for j in range(U_S1):
                base = (i * U_S1 + j) * 16
                outs = []
                for h in range(2):
                    r0 = pl.multiple_of(base + h * 8, 8)
                    rhs = _cat([load(r0, a) for a in range(NA)], 0).astype(BF16)
                    outs.append(_nn(l1_ref[...], rhs))
                    tick()
                r0 = pl.multiple_of(base, 16)
                for k in range(NK):
                    re = _cat([o[k * 8:k * 8 + 8] for o in outs], 0)
                    im = _cat([o[128 + k * 8:128 + k * 8 + 8] for o in outs], 0)
                    dst[k * 3, pl.ds(r0, 16), :] = re.astype(BF16)
                    dst[k * 3 + 1, pl.ds(r0, 16), :] = im.astype(BF16)
                    dst[k * 3 + 2, pl.ds(r0, 16), :] = (re + im).astype(BF16)
            return carry
        lax.fori_loop(0, D // 16 // U_S1, body, 0)

    def k_finish():
        cp_g.wait()
        for a in range(2, NA):
            c = 0 if a < 4 else (1 if a < 8 else 2)
            kt[a * D:(a + 1) * D, :] = _nn(kt[a * D:(a + 1) * D, :].astype(BF16), sel_ref[c])

        stage1(lambda r0, a: kt[pl.ds(a * D + r0, 8), :], s1k)

        def kf_body(i, carry):
            for kk in range(2):
                k = i * 2 + kk
                kf[2 * k], kf[2 * k + 1] = dft_fwd(s1k, k, slice(None))
            return carry
        lax.fori_loop(0, NK // 2, kf_body, 0)

    cp_g.start()

    def xin(i, carry):
        cp_x(i).wait()
        c0 = pl.multiple_of(i * TS, TS)
        xt[:, pl.ds(c0, TS)] = x_ref[pl.ds(c0, TS), :].astype(F32).T
        return carry
    lax.fori_loop(0, NT, xin, 0)

    def softmax_pair(p):
        ps = [p[f * 8:(f + 1) * 8] for f in range(16)]
        mx = functools.reduce(jnp.maximum, ps)
        mn = functools.reduce(jnp.minimum, ps)
        ep = [jnp.exp2(t - mx) for t in ps]
        en = [jnp.exp2(mn - t) for t in ps]
        rp = 1.0 / functools.reduce(jnp.add, ep)
        rn = 1.0 / functools.reduce(jnp.add, en)
        return _cat([t * rp for t in ep] + [t * rn for t in en], 0)

    def ln_to_ub(i, slot):
        c0 = pl.multiple_of(i * TS, TS)
        for h in range(NH):
            u = _layernorm_t(xt[:, pl.ds(c0 + h * 128, 128)]).astype(BF16)
            ub[slot * NH + h] = u

    def layer_a(with_kgen):
        ln_to_ub(0, 0)

        def p1(i, carry):
            slot = i % 2
            tick = Ticker(i * KP1, KP1, 48) if with_kgen else no_tick
            for g in range(4):
                if g == 2:
                    ln_to_ub(jnp.minimum(i + 1, NT - 1), 1 - slot)
                for h in range(NH):
                    n = g * NH + h
                    t = i * NH + h

                    def proj(j):
                        r0 = g * 384 + j * 128
                        w = _cat([wt[kk, r0:r0 + 128, :] for kk in range(4)], 1)
                        return _nn(w, ub[slot * NH + h])

                    pq = proj(0)
                    tick()
                    pk = proj(1)
                    tick()
                    phiq[t, g * 256:(g + 1) * 256, :] = softmax_pair(pq).astype(BF16)
                    pv = proj(2)
                    tick()
                    phik[t, g * 256:(g + 1) * 256, :] = softmax_pair(pk).astype(BF16)
                    vt[t, g * 128:(g + 1) * 128, :] = pv.astype(BF16)
            return carry
        lax.fori_loop(0, NT, p1, 0)

        rowi = lax.broadcasted_iota(jnp.int32, (144, 256), 0)
        coli = lax.broadcasted_iota(jnp.int32, (144, 256), 1)
        kvmask = (rowi % 8 == coli % 8) & (rowi < 136)
        ones = jnp.ones((16, 128), BF16)

        def kv_body(g, carry):
            tick = Ticker(4 * KP1 + g * KKV, KKV, 16) if with_kgen else no_tick
            acc = None
            for c in range(S // 128):
                lhs = _cat([vt[c, pl.ds(pl.multiple_of(g * 128, 128), 128), :], ones], 0)
                r = _nt(lhs, phik[c, pl.ds(pl.multiple_of(g * 256, 256), 256), :])
                acc = r if acc is None else acc + r
                tick()
            t = jnp.where(kvmask, acc, 0.0).astype(BF16)
            kvl[g * 2] = t[:, 0:128]
            kvl[g * 2 + 1] = t[:, 128:256]
            return carry
        lax.fori_loop(0, 4, kv_body, 0)

        NP2 = 4 if with_kgen else 8

        def p2(i, carry):
            tick = Ticker(4 * (KP1 + KKV) + i * KP2, KP2, 5 * NP2) if with_kgen else no_tick

            def num(h):
                os_ = []
                for g in range(4):
                    nd = _nn(_cat([kvl[g * 2], kvl[g * 2 + 1]], 1),
                             phiq[i * NP2 + h, g * 256:(g + 1) * 256, :])
                    r = 1.0 / (nd[128:136] + 1e-6)
                    os_ += [nd[d * 8:(d + 1) * 8] * r for d in range(16)]
                    tick()
                return _cat(os_, 0).astype(BF16)

            def fin(h, o):
                c0 = pl.multiple_of((i * NP2 + h) * 128, 128)
                w = _cat([wot[g] for g in range(4)], 1)
                xn = xt[:, pl.ds(c0, 128)] + _nn(w, o)
                xt[:, pl.ds(c0, 128)] = xn
                ut[:, pl.ds(c0, 128)] = _layernorm_t(xn)
                tick()

            prev = num(0)
            for h in range(1, NP2):
                cur = num(h)
                fin(h - 1, prev)
                prev = cur
            fin(NP2 - 1, prev)
            return carry
        lax.fori_loop(0, S // 128 // NP2, p2, 0)

    def layer_b(first):
        def hook(i):
            return Ticker(4 * (KP1 + KKV + KP2) + i * KS1, KS1, 2 * U_S1)
        stage1(lambda r0, a: ut[pl.ds(r0, 8), a * 128:(a + 1) * 128], s1, hook if first else None)
        if first:
            k_finish()

        def mid(i, carry):
            items = [(i * U_MID + kk, c) for kk in range(U_MID) for c in range(D // RC)]

            def fwd(k, c):
                rows = pl.ds(c * RC, RC)
                zr_, zi_ = dft_fwd(s1, k, rows)
                yr, yi = _cmul(zr_, zi_, kf[2 * k, rows, :], kf[2 * k + 1, rows, :])
                return yr.astype(BF16), yi.astype(BF16), (yr + yi).astype(BF16)

            def inv(k, c, y):
                rows = pl.ds(c * RC, RC)
                j1 = _nt(y[2], g_ref[3 * k])
                s2[2 * k, rows, :] = j1 + _nt(y[1], g_ref[3 * k + 1])
                s2[2 * k + 1, rows, :] = j1 - _nt(y[0], g_ref[3 * k + 2])
            prev = fwd(*items[0])
            for n in range(1, len(items)):
                cur = fwd(*items[n])
                inv(*items[n - 1], prev)
                prev = cur
            inv(*items[-1], prev)
            return carry
        lax.fori_loop(0, NK // U_MID, mid, 0)

        def last(i, carry):
            for j in range(U_LAST):
                r0 = pl.multiple_of((i * U_LAST + j) * 8, 8)
                rhs = _cat([s2[2 * k + ri, pl.ds(r0, 8), :] for ri in range(2) for k in range(NK)],
                           0).astype(BF16)
                y = _nn(_cat([l1inv_ref[0], l1inv_ref[1]], 1), rhs)
                dk = dskb[pl.ds(r0, 8), :]
                for a in range(NA):
                    sl = (pl.ds(r0, 8), slice(a * 128, (a + 1) * 128))
                    xt[sl] = xt[sl] + (y[a * 8:(a + 1) * 8] + ut[sl] * dk)
            return carry
        lax.fori_loop(0, D // 8 // U_LAST, last, 0)

    layer_a(True)
    layer_b(True)
    layer_a(False)
    layer_b(False)

    def xout(i, carry):
        c0 = pl.multiple_of(i * TS, TS)
        o_ref[pl.ds(c0, TS), :] = xt[:, pl.ds(c0, TS)].T.astype(BF16)
        pltpu.make_async_copy(o_ref.at[pl.ds(c0, TS), :], o_hbm.at[pl.ds(c0, TS), :],
                              sems.at[4 + i]).start()
        return carry
    lax.fori_loop(0, NT, xout, 0)
    for i in range(NT):
        pltpu.make_async_copy(o_ref.at[pl.ds(i * TS, TS), :], o_hbm.at[pl.ds(i * TS, TS), :],
                              sems.at[4 + i]).wait()


def _run(A_x, A_wqkv, A_w_phi, A_wo, B_A_re, B_A_im, B_B_re, B_B_im, B_C_re, B_C_im,
         B_log_dt, B_Dskip, interpret=False):
    consts = [jnp.asarray(c, dtype=BF16) for c in (_L1, _L1INV, _G, _SEL, _E, _PERM)]
    scratch = [
        pltpu.VMEM((D, S), F32),
        pltpu.VMEM((D, S), F32),
        pltpu.VMEM((2 * TS // 128, D, 128), BF16),
        pltpu.VMEM((S // 128, 2 * D, 128), BF16),
        pltpu.VMEM((S // 128, 2 * D, 128), BF16),
        pltpu.VMEM((S // 128, D, 128), BF16),
        pltpu.VMEM((NK * 3, D, 128), BF16),
        pltpu.VMEM((NK * 3, D, 128), BF16),
        pltpu.VMEM((NK * 2, D, 128), F32),
        pltpu.VMEM((NK * 2, D, 128), F32),
        pltpu.VMEM((NA * D, 128), F32),
        pltpu.VMEM((12, D, NS), F32),
        pltpu.VMEM((12, D, NS), F32),
        pltpu.VMEM((4, 3 * D, 128), BF16),
        pltpu.VMEM((4, D, 128), BF16),
        pltpu.VMEM((D, 128), F32),
        pltpu.VMEM((8, 144, 128), BF16),
        pltpu.VMEM((S, D), BF16),
        pltpu.VMEM((D, 3 * D), BF16),
        pltpu.VMEM((D, D), BF16),
        pltpu.VMEM((NK * 3, 128, 128), BF16),
        pltpu.VMEM((S, D), BF16),
        pltpu.SemaphoreType.DMA((4 + 2 * (S // TS),)),
    ]
    out = pl.pallas_call(
        _kernel,
        out_shape=jax.ShapeDtypeStruct((S, D), BF16),
        in_specs=[pl.BlockSpec(memory_space=pl.ANY) if i in (0, 1, 3, 14)
                  else pl.BlockSpec(memory_space=pltpu.VMEM) for i in range(18)],
        out_specs=pl.BlockSpec(memory_space=pl.ANY),
        scratch_shapes=scratch,
        compiler_params=pltpu.CompilerParams(vmem_limit_bytes=110 * 2**20, flags=FLAGS),
        interpret=interpret,
        name="hedgehog_s4",
    )(A_x.reshape(S, D), A_wqkv, A_w_phi, A_wo, B_A_re, B_A_im, B_B_re,
      B_B_im, B_C_re, B_C_im, B_log_dt, B_Dskip, *consts)
    return out.reshape(1, S, D)


@jax.jit
def pallas_interleave_layers__linear_kernel_hedgehog__ssm_conv_s4__prompt_kernel(
    A_x: jax.Array,
    A_wqkv: jax.Array,
    A_w_phi: jax.Array,
    A_wo: jax.Array,
    B_u: jax.Array,
    B_A_re: jax.Array,
    B_A_im: jax.Array,
    B_B_re: jax.Array,
    B_B_im: jax.Array,
    B_C_re: jax.Array,
    B_C_im: jax.Array,
    B_log_dt: jax.Array,
    B_Dskip: jax.Array,
):
    del B_u
    return _run(A_x, A_wqkv, A_w_phi, A_wo, B_A_re, B_A_im, B_B_re, B_B_im,
                B_C_re, B_C_im, B_log_dt, B_Dskip)
```
